```python
import os as _os
_os.environ.setdefault("JAX_PLATFORMS", "cpu")
import jax
import jax.numpy as jnp

def _softmax(x, axis=-1):
    return jax.nn.softmax(x, axis=axis)
def _gelu(x):
    return jax.nn.gelu(x, approximate=True)
def _silu(x):
    return jax.nn.silu(x)
def _sigmoid(x):
    return jax.nn.sigmoid(x)
def _layernorm(x, axis=-1, eps=1e-5):
    m = jnp.mean(x, axis=axis, keepdims=True)
    v = jnp.var(x, axis=axis, keepdims=True)
    return (x - m) / jnp.sqrt(v + eps)
def _scatter_add(tgt, idx, src, axis=0):
    return tgt.at[idx].add(src)
def _segment_sum(src, seg, n):
    return jax.ops.segment_sum(src, seg, n)
class _Rng:
    def __init__(self, key):
        self._k = key
    def _next(self):
        self._k, sub = jax.random.split(self._k)
        return sub
    def normal(self, shape):
        return jax.random.normal(self._next(), shape, dtype=jnp.bfloat16)
    def randint(self, lo, hi, shape):
        return jax.random.randint(self._next(), shape, lo, hi, dtype=jnp.int32)
    def uniform(self, shape, lo=0.0, hi=1.0):
        return jax.random.uniform(self._next(), shape, jnp.bfloat16, lo, hi)
    def permutation(self, n):
        return jax.random.permutation(self._next(), n)


kernel_name = 'concat_heads__ssm_conv_s4__linear_attn_block__prompt'

def setup_inputs():
    _rng = _Rng(jax.random.key(int.from_bytes(__import__("os").urandom(4), "little")))
    _w = (lambda a: (lambda t: t.astype(jnp.bfloat16) if jnp.issubdtype(t.dtype, jnp.floating) else t)(jnp.asarray(a)))
    def _A_setup():
        B, L, D, N = 1, 2048, 512, 128
        A_re = -jnp.exp((lambda *s: _rng.normal(s) * 0.1)(D, N))
        A_im = jnp.pi * (lambda *s: _rng.normal(s) * 0.1)(D, N)
        B_re = (lambda *s: _rng.normal(s) * 0.1)(D, N)
        B_im = (lambda *s: _rng.normal(s) * 0.1)(D, N)
        C_re = (lambda *s: _rng.normal(s) * 0.1)(D, N)
        C_im = (lambda *s: _rng.normal(s) * 0.1)(D, N)
        log_dt = (lambda *s: _rng.normal(s) * 0.1)(D) * 0.5 - 4.0
        Dskip = (lambda *s: _rng.normal(s) * 0.05)(D)
        return {
            "u": _w((lambda *s: _rng.normal(s) * 0.05)(B, L, D)),
            "A_re": _w(A_re),
            "A_im": _w(A_im),
            "B_re": _w(B_re),
            "B_im": _w(B_im),
            "C_re": _w(C_re),
            "C_im": _w(C_im),
            "log_dt": _w(log_dt),
            "Dskip": _w(Dskip),
        }
    _A_in = _A_setup()

    def _B_setup():
        B, S, D = 1, 2048, 512
        return {
            "x": _w((lambda *s: _rng.normal(s) * 0.05)(B, S, D)),
            "wqkv": _w((lambda *s: _rng.normal(s) * 0.4)(D, 3 * D)),
            "wo": _w((lambda *s: _rng.normal(s) * 0.05)(D, D)),
        }
    _B_in = _B_setup()

    return {
        "A_u": _A_in["u"],
        "A_A_re": _A_in["A_re"],
        "A_A_im": _A_in["A_im"],
        "A_B_re": _A_in["B_re"],
        "A_B_im": _A_in["B_im"],
        "A_C_re": _A_in["C_re"],
        "A_C_im": _A_in["C_im"],
        "A_log_dt": _A_in["log_dt"],
        "A_Dskip": _A_in["Dskip"],
        "B_x": _B_in["x"],
        "B_wqkv": _B_in["wqkv"],
        "B_wo": _B_in["wo"],
    }

def reference(A_u, A_A_re, A_A_im, A_B_re, A_B_im, A_C_re, A_C_im, A_log_dt, A_Dskip, B_x, B_wqkv, B_wo):
    def _A_ref(u, A_re, A_im, B_re, B_im, C_re, C_im, log_dt, Dskip):
        Bsz, L, D = u.shape
        dt = jnp.exp(log_dt)[:, None]
        A = A_re + 1j * A_im
        Bc = B_re + 1j * B_im
        Cc = C_re + 1j * C_im
        logdA = dt * A
        dB = dt * Bc
        l = (lambda x, dt: x.astype(dt))(jnp.arange(L), A_re.dtype)
        P = jnp.exp(logdA[:, :, None] * l[None, None, :])
        K = jnp.einsum("dn,dnl,dn->dl", Cc, P, dB).real
        L2 = 2 * L
        Kp = jnp.pad(K, ((0, 0), (0, L)))
        up = (lambda x, *d: x.transpose(*d))(u, 0, 2, 1)
        up = jnp.pad(up, ((0, 0), (0, 0), (0, L)))
        Kf = (lambda x, axes=(-2,-1): jnp.fft.rfft2(x.astype(jnp.float32), axes=axes))(Kp[:, None, :], axes=(-2, -1))
        Uf = (lambda x, axes=(-2,-1): jnp.fft.rfft2(x.astype(jnp.float32), axes=axes))(up[:, :, None, :], axes=(-2, -1))
        Yf = Uf * Kf[None, :, :, :]
        y = (lambda x, s, axes=(-2,-1): jnp.fft.irfft2(x, s=s, axes=axes).astype(jnp.bfloat16))(Yf, (1, L2), axes=(-2, -1))[:, :, 0, :L]
        y = (lambda x, *d: x.transpose(*d))(y, 0, 2, 1) + u * Dskip[None, None, :]
        return y

    def _B_ref(x, wqkv, wo):
        B, S, D = x.shape
        H = 32; Dh = D // H
        qkv = (lambda x, *d: x.transpose(*d))((x @ wqkv).reshape(B, S, 3, H, Dh), 2, 0, 3, 1, 4)
        q, k, v = qkv[0], qkv[1], qkv[2]
        phi = lambda t: jnp.where(t > 0, t + 1, jnp.exp(t)) + 1e-6
        pq, pk = phi(q), phi(k)
        kv = jnp.einsum("bhsd,bhse->bhde", pk, v)
        z = jnp.einsum("bhsd->bhd", pk)
        num = jnp.einsum("bhqd,bhde->bhqe", pq, kv)
        den = jnp.einsum("bhqd,bhd->bhq", pq, z)[..., None] + 1e-6
        o = num / den
        return (lambda x, *d: x.transpose(*d))(o, 0, 2, 1, 3).reshape(B, S, D) @ wo

    a = _A_ref(A_u, A_A_re, A_A_im, A_B_re, A_B_im, A_C_re, A_C_im, A_log_dt, A_Dskip)
    b = _B_ref(B_x, B_wqkv, B_wo)
    return jnp.concatenate([a, b], axis=-1)
```

```python
import jax
import jax.numpy as jnp
import numpy as np
import ml_dtypes
from jax import lax
import jax.experimental.pallas as pl
import jax.experimental.pallas.tpu as pltpu

L = 2048
D = 512
N = 128
Q = 128
NC = L // Q
F32 = jnp.float32
BF16 = jnp.bfloat16


def _consts():
    w = np.pi * (2 * np.arange(Q) + 1) / (2 * Q)
    s = np.arange(Q)
    fu = np.concatenate([np.cos(np.outer(w, s)), -np.sin(np.outer(w, s))], 0)
    g = fu.T / Q
    lr = np.arange(L).astype(np.float32).astype(ml_dtypes.bfloat16).astype(np.int64)
    fk = np.zeros((NC, 2 * Q, 2 * Q))
    for m in range(NC):
        for tau in range(-Q + 1, Q):
            l = Q * m + tau
            if l < 0:
                continue
            col = lr[l] - Q * (m - 1)
            if col == 2 * Q:
                col = 2 * Q - 1
            fk[m, :Q, col] += np.cos(w * tau)
            fk[m, Q:, col] -= np.sin(w * tau)
    b = ml_dtypes.bfloat16
    return fu.astype(b), fk.astype(b), g.astype(b)


_FU, _FK, _G = _consts()


def _cmul(a, b):
    return a[0] * b[0] - a[1] * b[1], a[0] * b[1] + a[1] * b[0]


def _csq(a):
    t = a[0] * a[1]
    return a[0] * a[0] - a[1] * a[1], t + t


def _phi(t):
    return jnp.where(t > 0, t + 1.0, jnp.exp(t)) + 1e-6


def _nt(a, b):
    return lax.dot_general(a, b, (((1,), (1,)), ((), ())), preferred_element_type=F32)


def _kernel(u_ref, are_ref, aim_ref, bre_ref, bim_ref, cre_ref, cim_ref, ldt_ref, dsk_ref,
            x_ref, wqkv_ref, wo_ref, fu_ref, fk_ref, g_ref, out_ref,
            t1r, t1i, t2r, t2i, mul_ref, kbuf, kf, uf, ybuf, ystage, pq_ref, kv_ref, z_ref,
            ostage, sem_y, sem_o):
    c = pl.program_id(0)
    RB = L // 4

    @pl.when(c == 0)
    def _():
        kv_ref[...] = jnp.zeros_like(kv_ref)
        z_ref[...] = jnp.zeros_like(z_ref)

    x = x_ref[...]
    q = jnp.dot(x, wqkv_ref[:, 0:D], preferred_element_type=F32)
    pq_ref[pl.ds(pl.multiple_of(c * RB, RB), RB), :] = _phi(q).astype(BF16)
    pk = _phi(jnp.dot(x, wqkv_ref[:, D:2 * D], preferred_element_type=F32))
    z_ref[...] += jnp.sum(pk.reshape(RB // 8, 8, D), axis=0)
    pk = pk.astype(BF16)
    v = jnp.dot(x, wqkv_ref[:, 2 * D:3 * D], preferred_element_type=F32).astype(BF16)
    for t in range(4):
        sl = slice(128 * t, 128 * (t + 1))
        kv_ref[t] += lax.dot_general(pk[:, sl], v[:, sl], (((0,), (0,)), ((), ())),
                                     preferred_element_type=F32)

    dt = jnp.exp(ldt_ref[...].astype(F32)).astype(BF16).astype(F32)
    lr = dt * are_ref[...].astype(F32)
    li = dt * aim_ref[...].astype(F32)
    e = jnp.exp(lr)
    a = (e * jnp.cos(li), e * jnp.sin(li))
    wv = _cmul((cre_ref[...].astype(F32), cim_ref[...].astype(F32)),
               (dt * bre_ref[...].astype(F32), dt * bim_ref[...].astype(F32)))
    pw = {1: a}
    p = a
    for k in range(1, 12):
        p = _csq(p)
        pw[2 ** k] = p
    p = (jnp.ones_like(lr), jnp.zeros_like(lr))
    b = wv
    for qq in range(8):
        t2r[qq * 128:(qq + 1) * 128, :] = p[0]
        t2i[qq * 128:(qq + 1) * 128, :] = p[1]
        t1r[qq * 128:(qq + 1) * 128, :] = b[0]
        t1i[qq * 128:(qq + 1) * 128, :] = b[1]
        if qq < 7:
            p = _cmul(p, a)
            b = _cmul(b, pw[128])
    for k, key in enumerate((8, 64, 1024)):
        mul_ref[2 * k] = pw[key][0]
        mul_ref[2 * k + 1] = pw[key][1]
    kl = wv[0] * pw[2048][0] - wv[1] * pw[2048][1]
    klast = jnp.sum(kl, axis=1, keepdims=True)

    def kgen(gi, _):
        for dd in range(8):
            d = gi * 8 + dd
            row = lambda k: jnp.broadcast_to(mul_ref[k, pl.ds(d, 1), :], (8, N))
            m8, m64, m1024 = (row(0), row(1)), (row(2), row(3)), (row(4), row(5))
            st = pl.ds(d, 8, stride=128)
            p = (t2r[st, :], t2i[st, :])
            rows = [p]
            for _i in range(7):
                p = _cmul(p, m8)
                rows.append(p)
            e2 = jnp.concatenate(
                [jnp.concatenate([r[0] for r in rows], 0), jnp.concatenate([r[1] for r in rows], 0)],
                1).astype(BF16)
            b0 = (t1r[st, :], t1i[st, :])
            b1 = _cmul(b0, m1024)
            b2 = _cmul(b0, m64)
            b3 = _cmul(b1, m64)
            e1 = jnp.concatenate(
                [jnp.concatenate([b0[0], b1[0], b2[0], b3[0]], 0),
                 jnp.concatenate([-b0[1], -b1[1], -b2[1], -b3[1]], 0)], 1).astype(BF16)
            res = _nt(e1, e2)
            kbuf[pl.ds(d, NC, stride=128), :] = jnp.concatenate([res[:16], res[16:]], 1)
        return 0

    lax.fori_loop(0, 16, kgen, 0)

    lane = lax.broadcasted_iota(jnp.int32, (Q, Q), 1)

    def kchunk(j):
        kj = kbuf[j * Q:(j + 1) * Q, :]
        if j >= 2:
            nxt = klast if j == NC - 1 else kbuf[(j + 1) * Q:(j + 2) * Q, 0:1]
            kj = jnp.where(lane == Q - 1, nxt, kj)
        return kj.astype(BF16)

    prev = None
    for m in range(NC):
        cur = kchunk(m)
        r = _nt(fk_ref[m, :, Q:], cur)
        if m > 0:
            r = r + _nt(fk_ref[m, :, :Q], prev)
        prev = cur
        kf[0, m] = r[:Q]
        kf[1, m] = r[Q:] - r[:Q]
        kf[2, m] = r[Q:] + r[:Q]
        r = jnp.dot(fu_ref[...], u_ref[m * Q:(m + 1) * Q, :], preferred_element_type=F32)
        uf[0, m] = r[:Q] + r[Q:]
        uf[1, m] = r[:Q]
        uf[2, m] = r[Q:]

    def mac(fi, _):
        fs = pl.ds(pl.multiple_of(fi * 16, 16), 16)
        for i0 in range(0, NC, 2):
            acc = {}
            for j in range(i0 + 2):
                uu = [uf[t, j, fs, :] for t in range(3)]
                for i in (i0, i0 + 1):
                    if j <= i:
                        pr = [kf[t, i - j, fs, :] * uu[t] for t in range(3)]
                        acc[i] = pr if i not in acc else [x_ + y_ for x_, y_ in zip(acc[i], pr)]
            for i in (i0, i0 + 1):
                ybuf[i, fs, :] = (acc[i][0] - acc[i][2]).astype(BF16)
                ybuf[i, pl.ds(pl.multiple_of(Q + fi * 16, 16), 16), :] = (acc[i][0] + acc[i][1]).astype(BF16)
        return 0

    lax.fori_loop(0, Q // 16, mac, 0)

    def ycopy(cc):
        return pltpu.make_async_copy(
            ystage, out_ref.at[:, pl.ds(pl.multiple_of(cc * 128, 128), 128)], sem_y)

    @pl.when(c > 0)
    def _():
        ycopy(c - 1).wait()

    dsk = dsk_ref[...].astype(F32)
    for i in range(NC):
        y = jnp.dot(g_ref[...], ybuf[i], preferred_element_type=F32)
        ystage[i * Q:(i + 1) * Q, :] = (y + u_ref[i * Q:(i + 1) * Q, :].astype(F32) * dsk).astype(BF16)
    ycopy(c).start()

    @pl.when(c == 3)
    def _():
        r_i = lax.broadcasted_iota(jnp.int32, (128, 128), 0) // 16
        c_i = lax.broadcasted_iota(jnp.int32, (128, 128), 1) // 16
        msk = r_i == c_i
        z = jnp.sum(z_ref[...], axis=0, keepdims=True)
        zm, wc = [], []
        for t in range(4):
            sl = slice(128 * t, 128 * (t + 1))
            zt = jnp.broadcast_to(z[:, sl], (128, 128))
            zm.append(jnp.where(msk, zt, 0.0).astype(BF16))
            kvt = jnp.where(msk, kv_ref[t], 0.0).astype(BF16)
            wc.append(jnp.dot(kvt, wo_ref[sl, :], preferred_element_type=F32).astype(BF16))
        wcm = jnp.concatenate(wc, 0)
        for rb in range(4):
            pq = pq_ref[rb * RB:(rb + 1) * RB, :]
            o = []
            for t in range(4):
                pt = pq[:, 128 * t:128 * (t + 1)]
                den = _nt(pt, zm[t]) + 1e-6
                o.append((pt.astype(F32) / den).astype(BF16))
            o = jnp.concatenate(o, 1)
            ostage[rb] = jnp.dot(o, wcm, preferred_element_type=F32).astype(BF16)
            pltpu.make_async_copy(ostage.at[rb], out_ref.at[rb * RB:(rb + 1) * RB, D:2 * D],
                                  sem_o.at[rb]).start()
        for rb in range(4):
            pltpu.make_async_copy(ostage.at[rb], out_ref.at[rb * RB:(rb + 1) * RB, D:2 * D],
                                  sem_o.at[rb]).wait()
        ycopy(c).wait()


@jax.jit
def pallas_concat_heads__ssm_conv_s4__linear_attn_block__prompt_kernel(
    A_u, A_A_re, A_A_im, A_B_re, A_B_im, A_C_re, A_C_im, A_log_dt, A_Dskip, B_x, B_wqkv, B_wo,
):
    par = pl.BlockSpec((128, N), lambda c: (c, 0))
    full = lambda shp: pl.BlockSpec(shp, lambda c: (0,) * len(shp))
    out = pl.pallas_call(
        _kernel,
        grid=(4,),
        in_specs=[pl.BlockSpec((L, 128), lambda c: (0, c))] + [par] * 6 + [
            pl.BlockSpec((128, 1), lambda c: (c, 0)),
            pl.BlockSpec((1, 128), lambda c: (0, c)),
            pl.BlockSpec((L // 4, D), lambda c: (c, 0)),
            full((D, 3 * D)), full((D, D)), full(_FU.shape), full(_FK.shape), full(_G.shape)],
        out_specs=pl.BlockSpec(memory_space=pl.ANY),
        out_shape=jax.ShapeDtypeStruct((L, 2 * D), BF16),
        scratch_shapes=[pltpu.VMEM((8 * 128, N), F32)] * 4 + [
            pltpu.VMEM((6, 128, N), F32),
            pltpu.VMEM((NC * 128, Q), F32),
            pltpu.VMEM((3, NC, Q, 128), F32),
            pltpu.VMEM((3, NC, Q, 128), F32),
            pltpu.VMEM((NC, 2 * Q, 128), BF16),
            pltpu.VMEM((L, 128), BF16),
            pltpu.VMEM((L, D), BF16),
            pltpu.VMEM((4, 128, 128), F32),
            pltpu.VMEM((8, D), F32),
            pltpu.VMEM((4, L // 4, D), BF16),
            pltpu.SemaphoreType.DMA(()),
            pltpu.SemaphoreType.DMA((4,)),
        ],
        compiler_params=pltpu.CompilerParams(
            dimension_semantics=("arbitrary",), vmem_limit_bytes=100 * 1024 * 1024),
    )(A_u.reshape(L, D), A_A_re, A_A_im, A_B_re, A_B_im, A_C_re, A_C_im,
      A_log_dt.reshape(D, 1), A_Dskip.reshape(1, D), B_x.reshape(L, D), B_wqkv, B_wo,
      _FU, _FK, _G)
    return out.reshape(1, L, 2 * D)
```

```python
import jax
import jax.numpy as jnp
import numpy as np
import ml_dtypes
from jax import lax
import jax.experimental.pallas as pl
import jax.experimental.pallas.tpu as pltpu

L = 2048
D = 512
N = 128
Q = 128
NC = L // Q
F32 = jnp.float32
BF16 = jnp.bfloat16


def _consts():
    w = np.pi * (2 * np.arange(Q) + 1) / (2 * Q)
    s = np.arange(Q)
    fu = np.concatenate([np.cos(np.outer(w, s)), -np.sin(np.outer(w, s))], 0)
    g = fu.T / Q
    lr = np.arange(L).astype(np.float32).astype(ml_dtypes.bfloat16).astype(np.int64)
    fk = np.zeros((NC, 2 * Q, 2 * Q))
    for m in range(NC):
        for tau in range(-Q + 1, Q):
            l = Q * m + tau
            if l < 0:
                continue
            col = lr[l] - Q * (m - 1)
            if col == 2 * Q:
                col = 2 * Q - 1
            fk[m, :Q, col] += np.cos(w * tau)
            fk[m, Q:, col] -= np.sin(w * tau)
    b = ml_dtypes.bfloat16
    return fu.astype(b), fk.astype(b), g.astype(b)


_FU, _FK, _G = _consts()


def _cmul(a, b):
    return a[0] * b[0] - a[1] * b[1], a[0] * b[1] + a[1] * b[0]


def _csq(a):
    t = a[0] * a[1]
    return a[0] * a[0] - a[1] * a[1], t + t


def _phi(t):
    return jnp.where(t > 0, t + 1.0, jnp.exp(t)) + 1e-6


def _nt(a, b):
    return lax.dot_general(a, b, (((1,), (1,)), ((), ())), preferred_element_type=F32)


def _kernel(u_ref, are_ref, aim_ref, bre_ref, bim_ref, cre_ref, cim_ref, ldt_ref, dsk_ref,
            x_ref, wqkv_ref, wo_ref, fu_ref, fk_ref, g_ref, out_ref,
            t1r, t1i, t2r, t2i, mul_ref, kbuf, kf, uf, ybuf, ystage, pq_ref, kv_ref, z_ref,
            wc_ref, ostage, sem_y, sem_o):
    c = pl.program_id(0)
    RB = L // 4

    @pl.when(c == 0)
    def _():
        kv_ref[...] = jnp.zeros_like(kv_ref)
        z_ref[...] = jnp.zeros_like(z_ref)

    def bq(r):
        x = x_ref[r * 128:(r + 1) * 128, :]
        q = jnp.dot(x, wqkv_ref[:, 0:D], preferred_element_type=F32)
        pq_ref[pl.ds(pl.multiple_of(c * RB + r * 128, 128), 128), :] = _phi(q).astype(BF16)

    def bkv(r):
        x = x_ref[r * 128:(r + 1) * 128, :]
        pk = _phi(jnp.dot(x, wqkv_ref[:, D:2 * D], preferred_element_type=F32))
        z_ref[...] += jnp.sum(pk.reshape(16, 8, D), axis=0)
        pk = pk.astype(BF16)
        v = jnp.dot(x, wqkv_ref[:, 2 * D:3 * D], preferred_element_type=F32).astype(BF16)
        for t in range(4):
            sl = slice(128 * t, 128 * (t + 1))
            kv_ref[t] += lax.dot_general(pk[:, sl], v[:, sl], (((0,), (0,)), ((), ())),
                                         preferred_element_type=F32)

    dt = jnp.exp(ldt_ref[...].astype(F32)).astype(BF16).astype(F32)
    lr = dt * are_ref[...].astype(F32)
    li = dt * aim_ref[...].astype(F32)
    e = jnp.exp(lr)
    a = (e * jnp.cos(li), e * jnp.sin(li))
    wv = _cmul((cre_ref[...].astype(F32), cim_ref[...].astype(F32)),
               (dt * bre_ref[...].astype(F32), dt * bim_ref[...].astype(F32)))
    pw = {1: a}
    p = a
    for k in range(1, 12):
        p = _csq(p)
        pw[2 ** k] = p
    p = (jnp.ones_like(lr), jnp.zeros_like(lr))
    b = wv
    for qq in range(8):
        t2r[qq * 128:(qq + 1) * 128, :] = p[0]
        t2i[qq * 128:(qq + 1) * 128, :] = p[1]
        t1r[qq * 128:(qq + 1) * 128, :] = b[0]
        t1i[qq * 128:(qq + 1) * 128, :] = b[1]
        if qq < 7:
            p = _cmul(p, a)
            b = _cmul(b, pw[128])
    for k, key in enumerate((8, 64, 1024)):
        mul_ref[2 * k] = pw[key][0]
        mul_ref[2 * k + 1] = pw[key][1]
    kl = wv[0] * pw[2048][0] - wv[1] * pw[2048][1]
    klast = jnp.sum(kl, axis=1, keepdims=True)

    def kgen(gi, _):
        for dd in range(8):
            d = gi * 8 + dd
            row = lambda k: jnp.broadcast_to(mul_ref[k, pl.ds(d, 1), :], (8, N))
            m8, m64, m1024 = (row(0), row(1)), (row(2), row(3)), (row(4), row(5))
            st = pl.ds(d, 8, stride=128)
            p = (t2r[st, :], t2i[st, :])
            rows = [p]
            for _i in range(7):
                p = _cmul(p, m8)
                rows.append(p)
            e2 = jnp.concatenate(
                [jnp.concatenate([r[0] for r in rows], 0), jnp.concatenate([r[1] for r in rows], 0)],
                1).astype(BF16)
            b0 = (t1r[st, :], t1i[st, :])
            b1 = _cmul(b0, m1024)
            b2 = _cmul(b0, m64)
            b3 = _cmul(b1, m64)
            e1 = jnp.concatenate(
                [jnp.concatenate([b0[0], b1[0], b2[0], b3[0]], 0),
                 jnp.concatenate([-b0[1], -b1[1], -b2[1], -b3[1]], 0)], 1).astype(BF16)
            res = _nt(e1, e2)
            kbuf[pl.ds(d, NC, stride=128), :] = jnp.concatenate([res[:16], res[16:]], 1)
        return 0

    for gi in range(16):
        if gi % 4 == 0:
            bq(gi // 4)
        if gi % 8 == 2:
            bkv(gi // 8)
        kgen(gi, 0)

    lane = lax.broadcasted_iota(jnp.int32, (Q, Q), 1)

    def kchunk(j):
        kj = kbuf[j * Q:(j + 1) * Q, :]
        if j >= 2:
            nxt = klast if j == NC - 1 else kbuf[(j + 1) * Q:(j + 2) * Q, 0:1]
            kj = jnp.where(lane == Q - 1, nxt, kj)
        return kj.astype(BF16)

    prev = None
    for m in range(NC):
        cur = kchunk(m)
        r = _nt(fk_ref[m, :, Q:], cur)
        if m > 0:
            r = r + _nt(fk_ref[m, :, :Q], prev)
        prev = cur
        kf[0, m] = r[:Q]
        kf[1, m] = r[Q:] - r[:Q]
        kf[2, m] = r[Q:] + r[:Q]
        r = jnp.dot(fu_ref[...], u_ref[m * Q:(m + 1) * Q, :], preferred_element_type=F32)
        uf[0, m] = r[:Q] + r[Q:]
        uf[1, m] = r[:Q]
        uf[2, m] = r[Q:]

    def mac(fi, _):
        fs = pl.ds(fi * 16, 16)
        for i0 in range(0, NC, 2):
            acc = {}
            for j in range(i0 + 2):
                uu = [uf[t, j, fs, :] for t in range(3)]
                for i in (i0, i0 + 1):
                    if j <= i:
                        pr = [kf[t, i - j, fs, :] * uu[t] for t in range(3)]
                        acc[i] = pr if i not in acc else [x_ + y_ for x_, y_ in zip(acc[i], pr)]
            for i in (i0, i0 + 1):
                ybuf[i, fs, :] = (acc[i][0] - acc[i][2]).astype(BF16)
                ybuf[i, pl.ds(Q + fi * 16, 16), :] = (acc[i][0] + acc[i][1]).astype(BF16)
        return 0

    for fi in range(Q // 16):
        if fi % 4 == 0:
            bkv(2 + fi // 4)
        mac(fi, 0)

    def ycopy(cc):
        return pltpu.make_async_copy(
            ystage, out_ref.at[:, pl.ds(pl.multiple_of(cc * 128, 128), 128)], sem_y)

    @pl.when(c > 0)
    def _():
        ycopy(c - 1).wait()

    dsk = dsk_ref[...].astype(F32)
    for i in range(NC):
        y = jnp.dot(g_ref[...], ybuf[i], preferred_element_type=F32)
        ystage[i * Q:(i + 1) * Q, :] = (y + u_ref[i * Q:(i + 1) * Q, :].astype(F32) * dsk).astype(BF16)
    ycopy(c).start()

    @pl.when(c == 3)
    def _():
        r_i = lax.broadcasted_iota(jnp.int32, (128, 128), 0) // 16
        c_i = lax.broadcasted_iota(jnp.int32, (128, 128), 1) // 16
        msk = r_i == c_i
        z = jnp.sum(z_ref[...], axis=0, keepdims=True)
        zm, wc = [], []
        for t in range(4):
            sl = slice(128 * t, 128 * (t + 1))
            zt = jnp.broadcast_to(z[:, sl], (128, 128))
            zm.append(jnp.where(msk, zt, 0.0).astype(BF16))
            kvt = jnp.where(msk, kv_ref[t], 0.0).astype(BF16)
            wc.append(jnp.dot(kvt, wo_ref[sl, :], preferred_element_type=F32).astype(BF16))
        wcm = jnp.concatenate(wc, 0)
        wc_ref[...] = wcm
        for rb in range(4):
            for r in range(4):
                pq = pq_ref[rb * RB + r * 128:rb * RB + (r + 1) * 128, :]
                o = []
                for t in range(4):
                    pt = pq[:, 128 * t:128 * (t + 1)]
                    den = _nt(pt, zm[t]) + 1e-6
                    rc = pl.reciprocal(den, approx=True)
                    rc = rc * (2.0 - den * rc)
                    o.append((pt.astype(F32) * rc).astype(BF16))
                o = jnp.concatenate(o, 1)
                ostage[rb, r * 128:(r + 1) * 128, :] = jnp.dot(
                    o, wc_ref[...], preferred_element_type=F32).astype(BF16)
            pltpu.make_async_copy(ostage.at[rb], out_ref.at[rb * RB:(rb + 1) * RB, D:2 * D],
                                  sem_o.at[rb]).start()
        for rb in range(4):
            pltpu.make_async_copy(ostage.at[rb], out_ref.at[rb * RB:(rb + 1) * RB, D:2 * D],
                                  sem_o.at[rb]).wait()
        ycopy(c).wait()


@jax.jit
def pallas_concat_heads__ssm_conv_s4__linear_attn_block__prompt_kernel(
    A_u, A_A_re, A_A_im, A_B_re, A_B_im, A_C_re, A_C_im, A_log_dt, A_Dskip, B_x, B_wqkv, B_wo,
):
    par = pl.BlockSpec((128, N), lambda c: (c, 0))
    full = lambda shp: pl.BlockSpec(shp, lambda c: (0,) * len(shp))
    out = pl.pallas_call(
        _kernel,
        grid=(4,),
        in_specs=[pl.BlockSpec((L, 128), lambda c: (0, c))] + [par] * 6 + [
            pl.BlockSpec((128, 1), lambda c: (c, 0)),
            pl.BlockSpec((1, 128), lambda c: (0, c)),
            pl.BlockSpec((L // 4, D), lambda c: (c, 0)),
            full((D, 3 * D)), full((D, D)), full(_FU.shape), full(_FK.shape), full(_G.shape)],
        out_specs=pl.BlockSpec(memory_space=pl.ANY),
        out_shape=jax.ShapeDtypeStruct((L, 2 * D), BF16),
        scratch_shapes=[pltpu.VMEM((8 * 128, N), F32)] * 4 + [
            pltpu.VMEM((6, 128, N), F32),
            pltpu.VMEM((NC * 128, Q), F32),
            pltpu.VMEM((3, NC, Q, 128), F32),
            pltpu.VMEM((3, NC, Q, 128), F32),
            pltpu.VMEM((NC, 2 * Q, 128), BF16),
            pltpu.VMEM((L, 128), BF16),
            pltpu.VMEM((L, D), BF16),
            pltpu.VMEM((4, 128, 128), F32),
            pltpu.VMEM((8, D), F32),
            pltpu.VMEM((D, D), BF16),
            pltpu.VMEM((4, L // 4, D), BF16),
            pltpu.SemaphoreType.DMA(()),
            pltpu.SemaphoreType.DMA((4,)),
        ],
        compiler_params=pltpu.CompilerParams(
            dimension_semantics=("arbitrary",), vmem_limit_bytes=100 * 1024 * 1024),
    )(A_u.reshape(L, D), A_A_re, A_A_im, A_B_re, A_B_im, A_C_re, A_C_im,
      A_log_dt.reshape(D, 1), A_Dskip.reshape(1, D), B_x.reshape(L, D), B_wqkv, B_wo,
      _FU, _FK, _G)
    return out.reshape(1, L, 2 * D)
```

```python
import jax
import jax.numpy as jnp
import numpy as np
import ml_dtypes
from jax import lax
import jax.experimental.pallas as pl
import jax.experimental.pallas.tpu as pltpu

L = 2048
D = 512
N = 128
Q = 128
NC = L // Q
F32 = jnp.float32
BF16 = jnp.bfloat16


def _consts():
    w = np.pi * (2 * np.arange(Q) + 1) / (2 * Q)
    s = np.arange(Q)
    fu = np.concatenate([np.cos(np.outer(w, s)), -np.sin(np.outer(w, s))], 0)
    g = fu.T / Q
    lr = np.arange(L).astype(np.float32).astype(ml_dtypes.bfloat16).astype(np.int64)
    fk = np.zeros((NC, 2 * Q, 2 * Q))
    for m in range(NC):
        for tau in range(-Q + 1, Q):
            l = Q * m + tau
            if l < 0:
                continue
            col = lr[l] - Q * (m - 1)
            if col == 2 * Q:
                col = 2 * Q - 1
            fk[m, :Q, col] += np.cos(w * tau)
            fk[m, Q:, col] -= np.sin(w * tau)
    b = ml_dtypes.bfloat16
    return fu.astype(b), fk.astype(b), g.astype(b)


_FU, _FK, _G = _consts()


def _cmul(a, b):
    return a[0] * b[0] - a[1] * b[1], a[0] * b[1] + a[1] * b[0]


def _csq(a):
    t = a[0] * a[1]
    return a[0] * a[0] - a[1] * a[1], t + t


def _phi(t):
    return jnp.where(t > 0, t + 1.0, jnp.exp(t)) + 1e-6


def _nt(a, b):
    return lax.dot_general(a, b, (((1,), (1,)), ((), ())), preferred_element_type=F32)


def _kernel(u_ref, are_ref, aim_ref, bre_ref, bim_ref, cre_ref, cim_ref, ldt_ref, dsk_ref,
            x_ref, wqkv_ref, wo_ref, fu_ref, fk_ref, g_ref, out_ref,
            t1r, t1i, t2r, t2i, mul_ref, kbuf, kf, uf, ybuf, ystage, pq_ref, kv_ref, z_ref,
            ws_ref, xs_ref, wc_ref, ostage, sem_y, sem_o):
    c = pl.program_id(0)
    RB = L // 4

    @pl.when(c == 0)
    def _():
        kv_ref[...] = jnp.zeros_like(kv_ref)
        z_ref[...] = jnp.zeros_like(z_ref)
        ws_ref[...] = wqkv_ref[...]

    xs_ref[...] = x_ref[...]

    def bq(r):
        x = xs_ref[pl.ds(pl.multiple_of(r * 128, 128), 128), :]
        q = jnp.dot(x, ws_ref[:, 0:D], preferred_element_type=F32)
        pq_ref[pl.ds(pl.multiple_of(c * RB + r * 128, 128), 128), :] = _phi(q).astype(BF16)

    def bkv(r):
        x = xs_ref[pl.ds(pl.multiple_of(r * 128, 128), 128), :]
        pk = _phi(jnp.dot(x, ws_ref[:, D:2 * D], preferred_element_type=F32))
        z_ref[...] += jnp.sum(pk.reshape(16, 8, D), axis=0)
        pk = pk.astype(BF16)
        v = jnp.dot(x, ws_ref[:, 2 * D:3 * D], preferred_element_type=F32).astype(BF16)
        for t in range(4):
            sl = slice(128 * t, 128 * (t + 1))
            kv_ref[t] += lax.dot_general(pk[:, sl], v[:, sl], (((0,), (0,)), ((), ())),
                                         preferred_element_type=F32)

    dt = jnp.exp(ldt_ref[...].astype(F32)).astype(BF16).astype(F32)
    lr = dt * are_ref[...].astype(F32)
    li = dt * aim_ref[...].astype(F32)
    e = jnp.exp(lr)
    a = (e * jnp.cos(li), e * jnp.sin(li))
    wv = _cmul((cre_ref[...].astype(F32), cim_ref[...].astype(F32)),
               (dt * bre_ref[...].astype(F32), dt * bim_ref[...].astype(F32)))
    pw = {1: a}
    p = a
    for k in range(1, 12):
        p = _csq(p)
        pw[2 ** k] = p
    p = (jnp.ones_like(lr), jnp.zeros_like(lr))
    b = wv
    for qq in range(8):
        t2r[qq * 128:(qq + 1) * 128, :] = p[0]
        t2i[qq * 128:(qq + 1) * 128, :] = p[1]
        t1r[qq * 128:(qq + 1) * 128, :] = b[0]
        t1i[qq * 128:(qq + 1) * 128, :] = b[1]
        if qq < 7:
            p = _cmul(p, a)
            b = _cmul(b, pw[128])
    for k, key in enumerate((8, 64, 1024)):
        mul_ref[2 * k] = pw[key][0]
        mul_ref[2 * k + 1] = pw[key][1]
    kl = wv[0] * pw[2048][0] - wv[1] * pw[2048][1]
    klast = jnp.sum(kl, axis=1, keepdims=True)

    def kgen(gi, _):
        for dd in range(8):
            d = gi * 8 + dd
            row = lambda k: jnp.broadcast_to(mul_ref[k, pl.ds(d, 1), :], (8, N))
            m8, m64, m1024 = (row(0), row(1)), (row(2), row(3)), (row(4), row(5))
            st = pl.ds(d, 8, stride=128)
            p = (t2r[st, :], t2i[st, :])
            rows = [p]
            for _i in range(7):
                p = _cmul(p, m8)
                rows.append(p)
            e2 = jnp.concatenate(
                [jnp.concatenate([r[0] for r in rows], 0), jnp.concatenate([r[1] for r in rows], 0)],
                1).astype(BF16)
            b0 = (t1r[st, :], t1i[st, :])
            b1 = _cmul(b0, m1024)
            b2 = _cmul(b0, m64)
            b3 = _cmul(b1, m64)
            e1 = jnp.concatenate(
                [jnp.concatenate([b0[0], b1[0], b2[0], b3[0]], 0),
                 jnp.concatenate([-b0[1], -b1[1], -b2[1], -b3[1]], 0)], 1).astype(BF16)
            res = _nt(e1, e2)
            kbuf[pl.ds(d, NC, stride=128), :] = jnp.concatenate([res[:16], res[16:]], 1)
        return 0

    for gi in range(16):
        if gi % 4 == 0:
            bq(gi // 4)
        if gi % 8 == 2:
            bkv(gi // 8)
        kgen(gi, 0)

    lane = lax.broadcasted_iota(jnp.int32, (Q, Q), 1)

    def kchunk(j):
        kj = kbuf[j * Q:(j + 1) * Q, :]
        if j >= 2:
            nxt = klast if j == NC - 1 else kbuf[(j + 1) * Q:(j + 2) * Q, 0:1]
            kj = jnp.where(lane == Q - 1, nxt, kj)
        return kj.astype(BF16)

    prev = None
    for m in range(NC):
        cur = kchunk(m)
        r = _nt(fk_ref[m, :, Q:], cur)
        if m > 0:
            r = r + _nt(fk_ref[m, :, :Q], prev)
        prev = cur
        kf[0, m] = r[:Q]
        kf[1, m] = r[Q:] - r[:Q]
        kf[2, m] = r[Q:] + r[:Q]
        r = jnp.dot(fu_ref[...], u_ref[m * Q:(m + 1) * Q, :], preferred_element_type=F32)
        uf[0, m] = r[:Q] + r[Q:]
        uf[1, m] = r[:Q]
        uf[2, m] = r[Q:]

    def mac(fi):
        IB = 4
        for i0 in range(0, NC, IB):
            res = []
            for h in range(2):
                fs = pl.ds(pl.multiple_of(fi * 16 + h * 8, 8), 8)
                acc = {}
                kk = {}
                for j in range(i0 + IB - 1, -1, -1):
                    uu = [uf[t, j, fs, :] for t in range(3)]
                    for i in range(i0, i0 + IB):
                        if j <= i:
                            m = i - j
                            if m not in kk:
                                kk[m] = [kf[t, m, fs, :] for t in range(3)]
                            pr = [kk[m][t] * uu[t] for t in range(3)]
                            acc[i] = pr if i not in acc else [x_ + y_ for x_, y_ in zip(acc[i], pr)]
                res.append({i: (a_[0] - a_[2], a_[0] + a_[1]) for i, a_ in acc.items()})
            for i in range(i0, i0 + IB):
                for k in range(2):
                    ybuf[i, pl.ds(pl.multiple_of(k * Q + fi * 16, 16), 16), :] = jnp.concatenate(
                        [res[0][i][k], res[1][i][k]], 0).astype(BF16)

    def macloop(it, _):
        bkv(2 + it)
        for k in range(4):
            mac(it * 4 + k)
        return 0

    lax.fori_loop(0, 2, macloop, 0)

    def ycopy(cc):
        return pltpu.make_async_copy(
            ystage, out_ref.at[:, pl.ds(pl.multiple_of(cc * 128, 128), 128)], sem_y)

    @pl.when(c > 0)
    def _():
        ycopy(c - 1).wait()

    dsk = dsk_ref[...].astype(F32)
    for i in range(NC):
        y = jnp.dot(g_ref[...], ybuf[i], preferred_element_type=F32)
        ystage[i * Q:(i + 1) * Q, :] = (y + u_ref[i * Q:(i + 1) * Q, :].astype(F32) * dsk).astype(BF16)
    ycopy(c).start()

    @pl.when(c == 3)
    def _():
        r_i = lax.broadcasted_iota(jnp.int32, (128, 128), 0) // 16
        c_i = lax.broadcasted_iota(jnp.int32, (128, 128), 1) // 16
        msk = r_i == c_i
        z = jnp.sum(z_ref[...], axis=0, keepdims=True)
        zm, wc = [], []
        for t in range(4):
            sl = slice(128 * t, 128 * (t + 1))
            zt = jnp.broadcast_to(z[:, sl], (128, 128))
            zm.append(jnp.where(msk, zt, 0.0).astype(BF16))
            kvt = jnp.where(msk, kv_ref[t], 0.0).astype(BF16)
            wc.append(jnp.dot(kvt, wo_ref[sl, :], preferred_element_type=F32).astype(BF16))
        wcm = jnp.concatenate(wc, 0)
        wc_ref[...] = wcm
        for rb in range(4):
            for r in range(4):
                pq = pq_ref[rb * RB + r * 128:rb * RB + (r + 1) * 128, :]
                o = []
                for t in range(4):
                    pt = pq[:, 128 * t:128 * (t + 1)]
                    den = _nt(pt, zm[t]) + 1e-6
                    rc = pl.reciprocal(den, approx=True)
                    rc = rc * (2.0 - den * rc)
                    o.append((pt.astype(F32) * rc).astype(BF16))
                o = jnp.concatenate(o, 1)
                ostage[rb, r * 128:(r + 1) * 128, :] = jnp.dot(
                    o, wc_ref[...], preferred_element_type=F32).astype(BF16)
            pltpu.make_async_copy(ostage.at[rb], out_ref.at[rb * RB:(rb + 1) * RB, D:2 * D],
                                  sem_o.at[rb]).start()
        for rb in range(4):
            pltpu.make_async_copy(ostage.at[rb], out_ref.at[rb * RB:(rb + 1) * RB, D:2 * D],
                                  sem_o.at[rb]).wait()
        ycopy(c).wait()


@jax.jit
def pallas_concat_heads__ssm_conv_s4__linear_attn_block__prompt_kernel(
    A_u, A_A_re, A_A_im, A_B_re, A_B_im, A_C_re, A_C_im, A_log_dt, A_Dskip, B_x, B_wqkv, B_wo,
):
    par = pl.BlockSpec((128, N), lambda c: (c, 0))
    full = lambda shp: pl.BlockSpec(shp, lambda c: (0,) * len(shp))
    out = pl.pallas_call(
        _kernel,
        grid=(4,),
        in_specs=[pl.BlockSpec((L, 128), lambda c: (0, c))] + [par] * 6 + [
            pl.BlockSpec((128, 1), lambda c: (c, 0)),
            pl.BlockSpec((1, 128), lambda c: (0, c)),
            pl.BlockSpec((L // 4, D), lambda c: (c, 0)),
            full((D, 3 * D)), full((D, D)), full(_FU.shape), full(_FK.shape), full(_G.shape)],
        out_specs=pl.BlockSpec(memory_space=pl.ANY),
        out_shape=jax.ShapeDtypeStruct((L, 2 * D), BF16),
        scratch_shapes=[pltpu.VMEM((8 * 128, N), F32)] * 4 + [
            pltpu.VMEM((6, 128, N), F32),
            pltpu.VMEM((NC * 128, Q), F32),
            pltpu.VMEM((3, NC, Q, 128), F32),
            pltpu.VMEM((3, NC, Q, 128), F32),
            pltpu.VMEM((NC, 2 * Q, 128), BF16),
            pltpu.VMEM((L, 128), BF16),
            pltpu.VMEM((L, D), BF16),
            pltpu.VMEM((4, 128, 128), F32),
            pltpu.VMEM((8, D), F32),
            pltpu.VMEM((D, 3 * D), BF16),
            pltpu.VMEM((L // 4, D), BF16),
            pltpu.VMEM((D, D), BF16),
            pltpu.VMEM((4, L // 4, D), BF16),
            pltpu.SemaphoreType.DMA(()),
            pltpu.SemaphoreType.DMA((4,)),
        ],
        compiler_params=pltpu.CompilerParams(
            dimension_semantics=("arbitrary",), vmem_limit_bytes=100 * 1024 * 1024),
    )(A_u.reshape(L, D), A_A_re, A_A_im, A_B_re, A_B_im, A_C_re, A_C_im,
      A_log_dt.reshape(D, 1), A_Dskip.reshape(1, D), B_x.reshape(L, D), B_wqkv, B_wo,
      _FU, _FK, _G)
    return out.reshape(1, L, 2 * D)
```

```python
import jax
import jax.numpy as jnp
import numpy as np
import ml_dtypes
from jax import lax
import jax.experimental.pallas as pl
import jax.experimental.pallas.tpu as pltpu

L = 2048
D = 512
N = 128
Q = 128
NC = L // Q
F32 = jnp.float32
BF16 = jnp.bfloat16


def _consts():
    w = np.pi * (2 * np.arange(Q) + 1) / (2 * Q)
    s = np.arange(Q)
    fu = np.concatenate([np.cos(np.outer(w, s)), -np.sin(np.outer(w, s))], 0)
    g = fu.T / Q
    lr = np.arange(L).astype(np.float32).astype(ml_dtypes.bfloat16).astype(np.int64)
    fk = np.zeros((NC, 2 * Q, 2 * Q))
    for m in range(NC):
        for tau in range(-Q + 1, Q):
            l = Q * m + tau
            if l < 0:
                continue
            col = lr[l] - Q * (m - 1)
            if col == 2 * Q:
                col = 2 * Q - 1
            fk[m, :Q, col] += np.cos(w * tau)
            fk[m, Q:, col] -= np.sin(w * tau)
    b = ml_dtypes.bfloat16
    return fu.astype(b), fk.astype(b), g.astype(b)


_FU, _FK, _G = _consts()


def _cmul(a, b):
    return a[0] * b[0] - a[1] * b[1], a[0] * b[1] + a[1] * b[0]


def _csq(a):
    t = a[0] * a[1]
    return a[0] * a[0] - a[1] * a[1], t + t


def _phi(t):
    return jnp.where(t > 0, t + 1.0, jnp.exp(t)) + 1e-6


def _nt(a, b):
    return lax.dot_general(a, b, (((1,), (1,)), ((), ())), preferred_element_type=F32)


def _kernel(u_ref, are_ref, aim_ref, bre_ref, bim_ref, cre_ref, cim_ref, ldt_ref, dsk_ref,
            x_ref, wqkv_ref, wo_ref, fu_ref, fk_ref, g_ref, out_ref,
            t1r, t1i, t2r, t2i, mul_ref, kbuf, kf, uf, ybuf, ystage, pq_ref, kv_ref, z_ref,
            wc_ref, ostage, sem_y, sem_o):
    c = pl.program_id(0)
    RB = L // 4

    @pl.when(c == 0)
    def _():
        kv_ref[...] = jnp.zeros_like(kv_ref)
        z_ref[...] = jnp.zeros_like(z_ref)

    def bq(r, t):
        x = x_ref[pl.ds(pl.multiple_of(r * 128, 128), 128), :]
        sl = slice(128 * t, 128 * (t + 1))
        q = jnp.dot(x, wqkv_ref[:, sl], preferred_element_type=F32)
        pq_ref[pl.ds(pl.multiple_of(c * RB + r * 128, 128), 128), sl] = _phi(q).astype(BF16)

    def bkv(r, t):
        x = x_ref[pl.ds(pl.multiple_of(r * 128, 128), 128), :]
        sl = slice(128 * t, 128 * (t + 1))
        pk = _phi(jnp.dot(x, wqkv_ref[:, D + 128 * t:D + 128 * (t + 1)], preferred_element_type=F32))
        z_ref[:, sl] += jnp.sum(pk.reshape(16, 8, 128), axis=0)
        pk = pk.astype(BF16)
        v = jnp.dot(x, wqkv_ref[:, 2 * D + 128 * t:2 * D + 128 * (t + 1)],
                    preferred_element_type=F32).astype(BF16)
        kv_ref[t] += lax.dot_general(pk, v, (((0,), (0,)), ((), ())), preferred_element_type=F32)

    def ufwd(m):
        r = jnp.dot(fu_ref[...], u_ref[m * Q:(m + 1) * Q, :], preferred_element_type=F32)
        uf[0, m] = r[:Q] + r[Q:]
        uf[1, m] = r[:Q]
        uf[2, m] = r[Q:]

    dt = jnp.exp(ldt_ref[...].astype(F32)).astype(BF16).astype(F32)
    lr = dt * are_ref[...].astype(F32)
    li = dt * aim_ref[...].astype(F32)
    e = jnp.exp(lr)
    a = (e * jnp.cos(li), e * jnp.sin(li))
    wv = _cmul((cre_ref[...].astype(F32), cim_ref[...].astype(F32)),
               (dt * bre_ref[...].astype(F32), dt * bim_ref[...].astype(F32)))
    pw = {1: a}
    p = a
    for k in range(1, 12):
        p = _csq(p)
        pw[2 ** k] = p
    p = (jnp.ones_like(lr), jnp.zeros_like(lr))
    b = wv
    for qq in range(8):
        t2r[qq * 128:(qq + 1) * 128, :] = p[0]
        t2i[qq * 128:(qq + 1) * 128, :] = p[1]
        t1r[qq * 128:(qq + 1) * 128, :] = b[0]
        t1i[qq * 128:(qq + 1) * 128, :] = b[1]
        if qq < 7:
            p = _cmul(p, a)
            b = _cmul(b, pw[128])
    for k, key in enumerate((8, 64, 1024)):
        mul_ref[2 * k] = pw[key][0]
        mul_ref[2 * k + 1] = pw[key][1]
    kl = wv[0] * pw[2048][0] - wv[1] * pw[2048][1]
    klast = jnp.sum(kl, axis=1, keepdims=True)

    def kgen(gi, _):
        for dd in range(8):
            d = gi * 8 + dd
            row = lambda k: jnp.broadcast_to(mul_ref[k, pl.ds(d, 1), :], (8, N))
            m8, m64, m1024 = (row(0), row(1)), (row(2), row(3)), (row(4), row(5))
            st = pl.ds(d, 8, stride=128)
            p = (t2r[st, :], t2i[st, :])
            rows = [p]
            for _i in range(7):
                p = _cmul(p, m8)
                rows.append(p)
            e2 = jnp.concatenate(
                [jnp.concatenate([r[0] for r in rows], 0), jnp.concatenate([r[1] for r in rows], 0)],
                1).astype(BF16)
            b0 = (t1r[st, :], t1i[st, :])
            b1 = _cmul(b0, m1024)
            b2 = _cmul(b0, m64)
            b3 = _cmul(b1, m64)
            e1 = jnp.concatenate(
                [jnp.concatenate([b0[0], b1[0], b2[0], b3[0]], 0),
                 jnp.concatenate([-b0[1], -b1[1], -b2[1], -b3[1]], 0)], 1).astype(BF16)
            res = _nt(e1, e2)
            kbuf[pl.ds(d, NC, stride=128), :] = jnp.concatenate([res[:16], res[16:]], 1)
        return 0

    for gi in range(16):
        bq(gi // 4, gi % 4)
        if gi % 2 == 0:
            bkv(gi // 8, (gi % 8) // 2)
        ufwd(gi)
        kgen(gi, 0)

    lane = lax.broadcasted_iota(jnp.int32, (Q, Q), 1)

    def kchunk(j):
        kj = kbuf[j * Q:(j + 1) * Q, :]
        if j >= 2:
            nxt = klast if j == NC - 1 else pltpu.roll(kbuf[(j + 1) * Q:(j + 2) * Q, :], Q - 1, 1)
            kj = jnp.where(lane == Q - 1, nxt, kj)
        return kj.astype(BF16)

    prev = None
    for m in range(NC):
        cur = kchunk(m)
        r = _nt(fk_ref[m, :, Q:], cur)
        if m > 0:
            r = r + _nt(fk_ref[m, :, :Q], prev)
        prev = cur
        kf[0, m] = r[:Q]
        kf[1, m] = r[Q:] - r[:Q]
        kf[2, m] = r[Q:] + r[:Q]

    def mac(fi):
        IB = 4
        for i0 in range(0, NC, IB):
            res = []
            for h in range(2):
                fs = pl.ds(pl.multiple_of(fi * 16 + h * 8, 8), 8)
                acc = {}
                kk = {}
                for j in range(i0 + IB - 1, -1, -1):
                    uu = [uf[t, j, fs, :] for t in range(3)]
                    for i in range(i0, i0 + IB):
                        if j <= i:
                            m = i - j
                            if m not in kk:
                                kk[m] = [kf[t, m, fs, :] for t in range(3)]
                            pr = [kk[m][t] * uu[t] for t in range(3)]
                            acc[i] = pr if i not in acc else [x_ + y_ for x_, y_ in zip(acc[i], pr)]
                res.append({i: (a_[0] - a_[2], a_[0] + a_[1]) for i, a_ in acc.items()})
            for i in range(i0, i0 + IB):
                for k in range(2):
                    ybuf[i, pl.ds(pl.multiple_of(k * Q + fi * 16, 16), 16), :] = jnp.concatenate(
                        [res[0][i][k], res[1][i][k]], 0).astype(BF16)

    def macloop(it, _):
        for k in range(4):
            bkv(2 + it, k)
            mac(it * 4 + k)
        return 0

    lax.fori_loop(0, 2, macloop, 0)

    def ycopy(cc):
        return pltpu.make_async_copy(
            ystage, out_ref.at[:, pl.ds(pl.multiple_of(cc * 128, 128), 128)], sem_y)

    @pl.when(c > 0)
    def _():
        ycopy(c - 1).wait()

    dsk = dsk_ref[...].astype(F32)
    for i in range(NC):
        y = jnp.dot(g_ref[...], ybuf[i], preferred_element_type=F32)
        ystage[i * Q:(i + 1) * Q, :] = (y + u_ref[i * Q:(i + 1) * Q, :].astype(F32) * dsk).astype(BF16)
    ycopy(c).start()

    @pl.when(c == 3)
    def _():
        r_i = lax.broadcasted_iota(jnp.int32, (128, 128), 0) // 16
        c_i = lax.broadcasted_iota(jnp.int32, (128, 128), 1) // 16
        msk = r_i == c_i
        z = jnp.sum(z_ref[...], axis=0, keepdims=True)
        zm, wc = [], []
        for t in range(4):
            sl = slice(128 * t, 128 * (t + 1))
            zt = jnp.broadcast_to(z[:, sl], (128, 128))
            zm.append(jnp.where(msk, zt, 0.0).astype(BF16))
            kvt = jnp.where(msk, kv_ref[t], 0.0).astype(BF16)
            wc.append(jnp.dot(kvt, wo_ref[sl, :], preferred_element_type=F32).astype(BF16))
        wcm = jnp.concatenate(wc, 0)
        wc_ref[...] = wcm
        for rb in range(4):
            for r in range(4):
                pq = pq_ref[rb * RB + r * 128:rb * RB + (r + 1) * 128, :]
                o = []
                for t in range(4):
                    pt = pq[:, 128 * t:128 * (t + 1)]
                    den = _nt(pt, zm[t]) + 1e-6
                    rc = pl.reciprocal(den, approx=True)
                    rc = rc * (2.0 - den * rc)
                    o.append((pt.astype(F32) * rc).astype(BF16))
                o = jnp.concatenate(o, 1)
                ostage[rb, r * 128:(r + 1) * 128, :] = jnp.dot(
                    o, wc_ref[...], preferred_element_type=F32).astype(BF16)
            pltpu.make_async_copy(ostage.at[rb], out_ref.at[rb * RB:(rb + 1) * RB, D:2 * D],
                                  sem_o.at[rb]).start()
        for rb in range(4):
            pltpu.make_async_copy(ostage.at[rb], out_ref.at[rb * RB:(rb + 1) * RB, D:2 * D],
                                  sem_o.at[rb]).wait()
        ycopy(c).wait()


@jax.jit
def pallas_concat_heads__ssm_conv_s4__linear_attn_block__prompt_kernel(
    A_u, A_A_re, A_A_im, A_B_re, A_B_im, A_C_re, A_C_im, A_log_dt, A_Dskip, B_x, B_wqkv, B_wo,
):
    par = pl.BlockSpec((128, N), lambda c: (c, 0))
    full = lambda shp: pl.BlockSpec(shp, lambda c: (0,) * len(shp))
    out = pl.pallas_call(
        _kernel,
        grid=(4,),
        in_specs=[pl.BlockSpec((L, 128), lambda c: (0, c))] + [par] * 6 + [
            pl.BlockSpec((128, 1), lambda c: (c, 0)),
            pl.BlockSpec((1, 128), lambda c: (0, c)),
            pl.BlockSpec((L // 4, D), lambda c: (c, 0)),
            full((D, 3 * D)), full((D, D)), full(_FU.shape), full(_FK.shape), full(_G.shape)],
        out_specs=pl.BlockSpec(memory_space=pl.ANY),
        out_shape=jax.ShapeDtypeStruct((L, 2 * D), BF16),
        scratch_shapes=[pltpu.VMEM((8 * 128, N), F32)] * 4 + [
            pltpu.VMEM((6, 128, N), F32),
            pltpu.VMEM((NC * 128, Q), F32),
            pltpu.VMEM((3, NC, Q, 128), F32),
            pltpu.VMEM((3, NC, Q, 128), F32),
            pltpu.VMEM((NC, 2 * Q, 128), BF16),
            pltpu.VMEM((L, 128), BF16),
            pltpu.VMEM((L, D), BF16),
            pltpu.VMEM((4, 128, 128), F32),
            pltpu.VMEM((8, D), F32),
            pltpu.VMEM((D, D), BF16),
            pltpu.VMEM((4, L // 4, D), BF16),
            pltpu.SemaphoreType.DMA(()),
            pltpu.SemaphoreType.DMA((4,)),
        ],
        compiler_params=pltpu.CompilerParams(
            dimension_semantics=("arbitrary",), vmem_limit_bytes=100 * 1024 * 1024),
    )(A_u.reshape(L, D), A_A_re, A_A_im, A_B_re, A_B_im, A_C_re, A_C_im,
      A_log_dt.reshape(D, 1), A_Dskip.reshape(1, D), B_x.reshape(L, D), B_wqkv, B_wo,
      _FU, _FK, _G)
    return out.reshape(1, L, 2 * D)
```

```python
import jax
import jax.numpy as jnp
import numpy as np
import ml_dtypes
from jax import lax
import jax.experimental.pallas as pl
import jax.experimental.pallas.tpu as pltpu

L = 2048
D = 512
N = 128
Q = 128
NC = L // Q
F32 = jnp.float32
BF16 = jnp.bfloat16


def _consts():
    w = np.pi * (2 * np.arange(Q) + 1) / (2 * Q)
    s = np.arange(Q)
    fu = np.concatenate([np.cos(np.outer(w, s)), -np.sin(np.outer(w, s))], 0)
    g = fu.T / Q
    lr = np.arange(L).astype(np.float32).astype(ml_dtypes.bfloat16).astype(np.int64)
    fk = np.zeros((NC, 2 * Q, 2 * Q))
    for m in range(NC):
        for tau in range(-Q + 1, Q):
            l = Q * m + tau
            if l < 0:
                continue
            col = lr[l] - Q * (m - 1)
            if col == 2 * Q:
                col = 2 * Q - 1
            fk[m, :Q, col] += np.cos(w * tau)
            fk[m, Q:, col] -= np.sin(w * tau)
    b = ml_dtypes.bfloat16
    return fu.astype(b), fk.astype(b), g.astype(b)


_FU, _FK, _G = _consts()


def _cmul(a, b):
    return a[0] * b[0] - a[1] * b[1], a[0] * b[1] + a[1] * b[0]


def _csq(a):
    t = a[0] * a[1]
    return a[0] * a[0] - a[1] * a[1], t + t


def _phi(t):
    return jnp.where(t > 0, t + 1.0, jnp.exp(t)) + 1e-6


def _nt(a, b):
    return lax.dot_general(a, b, (((1,), (1,)), ((), ())), preferred_element_type=F32)


def _kernel(u_ref, are_ref, aim_ref, bre_ref, bim_ref, cre_ref, cim_ref, ldt_ref, dsk_ref,
            x_ref, wqkv_ref, wo_ref, fu_ref, fk_ref, g_ref, out_ref,
            t1r, t1i, t2r, t2i, mul_ref, kbuf, kf, uf, ybuf, ystage, pq_ref, kv_ref, z_ref,
            wc_ref, ostage, sem_y, sem_o):
    c = pl.program_id(0)
    RB = L // 4

    @pl.when(c == 0)
    def _():
        kv_ref[...] = jnp.zeros_like(kv_ref)
        z_ref[...] = jnp.zeros_like(z_ref)

    def bq(r):
        x = x_ref[r * 128:(r + 1) * 128, :]
        q = jnp.dot(x, wqkv_ref[:, 0:D], preferred_element_type=F32)
        pq_ref[pl.ds(pl.multiple_of(c * RB + r * 128, 128), 128), :] = _phi(q).astype(BF16)

    def bkv(r):
        x = x_ref[r * 128:(r + 1) * 128, :]
        pk = _phi(jnp.dot(x, wqkv_ref[:, D:2 * D], preferred_element_type=F32))
        z_ref[...] += jnp.sum(pk.reshape(16, 8, D), axis=0)
        pk = pk.astype(BF16)
        v = jnp.dot(x, wqkv_ref[:, 2 * D:3 * D], preferred_element_type=F32).astype(BF16)
        for t in range(4):
            sl = slice(128 * t, 128 * (t + 1))
            kv_ref[t] += lax.dot_general(pk[:, sl], v[:, sl], (((0,), (0,)), ((), ())),
                                         preferred_element_type=F32)

    def ufwd(m):
        r = jnp.dot(fu_ref[...], u_ref[m * Q:(m + 1) * Q, :], preferred_element_type=F32)
        uf[0, m] = r[:Q] + r[Q:]
        uf[1, m] = r[:Q]
        uf[2, m] = r[Q:]

    dt = jnp.exp(ldt_ref[...].astype(F32)).astype(BF16).astype(F32)
    lr = dt * are_ref[...].astype(F32)
    li = dt * aim_ref[...].astype(F32)
    e = jnp.exp(lr)
    a = (e * jnp.cos(li), e * jnp.sin(li))
    wv = _cmul((cre_ref[...].astype(F32), cim_ref[...].astype(F32)),
               (dt * bre_ref[...].astype(F32), dt * bim_ref[...].astype(F32)))
    pw = {1: a}
    p = a
    for k in range(1, 12):
        p = _csq(p)
        pw[2 ** k] = p
    p = (jnp.ones_like(lr), jnp.zeros_like(lr))
    b = wv
    for qq in range(8):
        t2r[qq * 128:(qq + 1) * 128, :] = p[0]
        t2i[qq * 128:(qq + 1) * 128, :] = p[1]
        t1r[qq * 128:(qq + 1) * 128, :] = b[0]
        t1i[qq * 128:(qq + 1) * 128, :] = b[1]
        if qq < 7:
            p = _cmul(p, a)
            b = _cmul(b, pw[128])
    for k, key in enumerate((8, 64, 1024)):
        mul_ref[2 * k] = pw[key][0]
        mul_ref[2 * k + 1] = pw[key][1]
    kl = wv[0] * pw[2048][0] - wv[1] * pw[2048][1]
    klast = jnp.sum(kl, axis=1, keepdims=True)

    def kgen(gi, _):
        for dd in range(8):
            d = gi * 8 + dd
            row = lambda k: jnp.broadcast_to(mul_ref[k, pl.ds(d, 1), :], (8, N))
            m8, m64, m1024 = (row(0), row(1)), (row(2), row(3)), (row(4), row(5))
            st = pl.ds(d, 8, stride=128)
            p = (t2r[st, :], t2i[st, :])
            rows = [p]
            for _i in range(7):
                p = _cmul(p, m8)
                rows.append(p)
            e2 = jnp.concatenate(
                [jnp.concatenate([r[0] for r in rows], 0), jnp.concatenate([r[1] for r in rows], 0)],
                1).astype(BF16)
            b0 = (t1r[st, :], t1i[st, :])
            b1 = _cmul(b0, m1024)
            b2 = _cmul(b0, m64)
            b3 = _cmul(b1, m64)
            e1 = jnp.concatenate(
                [jnp.concatenate([b0[0], b1[0], b2[0], b3[0]], 0),
                 jnp.concatenate([-b0[1], -b1[1], -b2[1], -b3[1]], 0)], 1).astype(BF16)
            res = _nt(e1, e2)
            kbuf[pl.ds(d, NC, stride=128), :] = jnp.concatenate([res[:16], res[16:]], 1)
        return 0

    for gi in range(16):
        if gi % 4 == 0:
            bq(gi // 4)
        if gi % 4 == 2:
            for m in range(gi - 2, gi + 2):
                ufwd(m)
        kgen(gi, 0)

    lane = lax.broadcasted_iota(jnp.int32, (Q, Q), 1)

    def kchunk(j):
        kj = kbuf[j * Q:(j + 1) * Q, :]
        if j >= 2:
            nxt = klast if j == NC - 1 else pltpu.roll(kbuf[(j + 1) * Q:(j + 2) * Q, :], Q - 1, 1)
            kj = jnp.where(lane == Q - 1, nxt, kj)
        return kj.astype(BF16)

    prev = None
    for m in range(NC):
        cur = kchunk(m)
        r = _nt(fk_ref[m, :, Q:], cur)
        if m > 0:
            r = r + _nt(fk_ref[m, :, :Q], prev)
        prev = cur
        kf[0, m] = r[:Q]
        kf[1, m] = r[Q:] - r[:Q]
        kf[2, m] = r[Q:] + r[:Q]

    def mac(fi):
        IB = 4
        for i0 in range(0, NC, IB):
            res = []
            for h in range(2):
                fs = pl.ds(fi * 16 + h * 8, 8)
                acc = {}
                kk = {}
                for j in range(i0 + IB - 1, -1, -1):
                    uu = [uf[t, j, fs, :] for t in range(3)]
                    for i in range(i0, i0 + IB):
                        if j <= i:
                            m = i - j
                            if m not in kk:
                                kk[m] = [kf[t, m, fs, :] for t in range(3)]
                            pr = [kk[m][t] * uu[t] for t in range(3)]
                            acc[i] = pr if i not in acc else [x_ + y_ for x_, y_ in zip(acc[i], pr)]
                res.append({i: (a_[0] - a_[2], a_[0] + a_[1]) for i, a_ in acc.items()})
            for i in range(i0, i0 + IB):
                for k in range(2):
                    ybuf[i, pl.ds(k * Q + fi * 16, 16), :] = jnp.concatenate(
                        [res[0][i][k], res[1][i][k]], 0).astype(BF16)

    for fi in range(8):
        if fi % 2 == 0:
            bkv(fi // 2)
        mac(fi)

    def ycopy(cc):
        return pltpu.make_async_copy(
            ystage, out_ref.at[:, pl.ds(pl.multiple_of(cc * 128, 128), 128)], sem_y)

    @pl.when(c > 0)
    def _():
        ycopy(c - 1).wait()

    dsk = dsk_ref[...].astype(F32)
    for i in range(NC):
        y = jnp.dot(g_ref[...], ybuf[i], preferred_element_type=F32)
        ystage[i * Q:(i + 1) * Q, :] = (y + u_ref[i * Q:(i + 1) * Q, :].astype(F32) * dsk).astype(BF16)
    ycopy(c).start()

    @pl.when(c == 3)
    def _():
        r_i = lax.broadcasted_iota(jnp.int32, (128, 128), 0) // 16
        c_i = lax.broadcasted_iota(jnp.int32, (128, 128), 1) // 16
        msk = r_i == c_i
        z = jnp.sum(z_ref[...], axis=0, keepdims=True)
        zm, wc = [], []
        for t in range(4):
            sl = slice(128 * t, 128 * (t + 1))
            zt = jnp.broadcast_to(z[:, sl], (128, 128))
            zm.append(jnp.where(msk, zt, 0.0).astype(BF16))
            kvt = jnp.where(msk, kv_ref[t], 0.0).astype(BF16)
            wc.append(jnp.dot(kvt, wo_ref[sl, :], preferred_element_type=F32).astype(BF16))
        wcm = jnp.concatenate(wc, 0)
        wc_ref[...] = wcm
        for rb in range(4):
            for r in range(4):
                pq = pq_ref[rb * RB + r * 128:rb * RB + (r + 1) * 128, :]
                o = []
                for t in range(4):
                    pt = pq[:, 128 * t:128 * (t + 1)]
                    den = _nt(pt, zm[t]) + 1e-6
                    rc = pl.reciprocal(den, approx=True)
                    rc = rc * (2.0 - den * rc)
                    o.append((pt.astype(F32) * rc).astype(BF16))
                o = jnp.concatenate(o, 1)
                ostage[rb, r * 128:(r + 1) * 128, :] = jnp.dot(
                    o, wc_ref[...], preferred_element_type=F32).astype(BF16)
            pltpu.make_async_copy(ostage.at[rb], out_ref.at[rb * RB:(rb + 1) * RB, D:2 * D],
                                  sem_o.at[rb]).start()
        for rb in range(4):
            pltpu.make_async_copy(ostage.at[rb], out_ref.at[rb * RB:(rb + 1) * RB, D:2 * D],
                                  sem_o.at[rb]).wait()
        ycopy(c).wait()


@jax.jit
def pallas_concat_heads__ssm_conv_s4__linear_attn_block__prompt_kernel(
    A_u, A_A_re, A_A_im, A_B_re, A_B_im, A_C_re, A_C_im, A_log_dt, A_Dskip, B_x, B_wqkv, B_wo,
):
    par = pl.BlockSpec((128, N), lambda c: (c, 0))
    full = lambda shp: pl.BlockSpec(shp, lambda c: (0,) * len(shp))
    out = pl.pallas_call(
        _kernel,
        grid=(4,),
        in_specs=[pl.BlockSpec((L, 128), lambda c: (0, c))] + [par] * 6 + [
            pl.BlockSpec((128, 1), lambda c: (c, 0)),
            pl.BlockSpec((1, 128), lambda c: (0, c)),
            pl.BlockSpec((L // 4, D), lambda c: (c, 0)),
            full((D, 3 * D)), full((D, D)), full(_FU.shape), full(_FK.shape), full(_G.shape)],
        out_specs=pl.BlockSpec(memory_space=pl.ANY),
        out_shape=jax.ShapeDtypeStruct((L, 2 * D), BF16),
        scratch_shapes=[pltpu.VMEM((8 * 128, N), F32)] * 4 + [
            pltpu.VMEM((6, 128, N), F32),
            pltpu.VMEM((NC * 128, Q), F32),
            pltpu.VMEM((3, NC, Q, 128), F32),
            pltpu.VMEM((3, NC, Q, 128), F32),
            pltpu.VMEM((NC, 2 * Q, 128), BF16),
            pltpu.VMEM((L, 128), BF16),
            pltpu.VMEM((L, D), BF16),
            pltpu.VMEM((4, 128, 128), F32),
            pltpu.VMEM((8, D), F32),
            pltpu.VMEM((D, D), BF16),
            pltpu.VMEM((4, L // 4, D), BF16),
            pltpu.SemaphoreType.DMA(()),
            pltpu.SemaphoreType.DMA((4,)),
        ],
        compiler_params=pltpu.CompilerParams(
            dimension_semantics=("arbitrary",), vmem_limit_bytes=100 * 1024 * 1024),
    )(A_u.reshape(L, D), A_A_re, A_A_im, A_B_re, A_B_im, A_C_re, A_C_im,
      A_log_dt.reshape(D, 1), A_Dskip.reshape(1, D), B_x.reshape(L, D), B_wqkv, B_wo,
      _FU, _FK, _G)
    return out.reshape(1, L, 2 * D)
```

```python
import jax
import jax.numpy as jnp
import numpy as np
import ml_dtypes
from jax import lax
import jax.experimental.pallas as pl
import jax.experimental.pallas.tpu as pltpu

L = 2048
D = 512
N = 128
Q = 128
NC = L // Q
F32 = jnp.float32
BF16 = jnp.bfloat16


def _consts():
    w = np.pi * (2 * np.arange(Q) + 1) / (2 * Q)
    s = np.arange(Q)
    fu = np.concatenate([np.cos(np.outer(w, s)), -np.sin(np.outer(w, s))], 0)
    g = fu.T / Q
    lr = np.arange(L).astype(np.float32).astype(ml_dtypes.bfloat16).astype(np.int64)
    fk = np.zeros((NC, 2 * Q, 2 * Q))
    for m in range(NC):
        for tau in range(-Q + 1, Q):
            l = Q * m + tau
            if l < 0:
                continue
            col = lr[l] - Q * (m - 1)
            if col == 2 * Q:
                col = 2 * Q - 1
            fk[m, :Q, col] += np.cos(w * tau)
            fk[m, Q:, col] -= np.sin(w * tau)
    b = ml_dtypes.bfloat16
    return fu.astype(b), fk.astype(b), g.astype(b)


_FU, _FK, _G = _consts()


def _cmul(a, b):
    return a[0] * b[0] - a[1] * b[1], a[0] * b[1] + a[1] * b[0]


def _csq(a):
    t = a[0] * a[1]
    return a[0] * a[0] - a[1] * a[1], t + t


def _phi(t):
    return jnp.where(t > 0, t + 1.0, jnp.exp(t)) + 1e-6


def _nt(a, b):
    return lax.dot_general(a, b, (((1,), (1,)), ((), ())), preferred_element_type=F32)


def _kernel(u_ref, are_ref, aim_ref, bre_ref, bim_ref, cre_ref, cim_ref, ldt_ref, dsk_ref,
            x_ref, wqkv_ref, wo_ref, fu_ref, fk_ref, g_ref, out_ref,
            t1r, t1i, t2r, t2i, mul_ref, kbuf, kf, uf, ybuf, ystage, pq_ref, kv_ref, z_ref,
            wc_ref, ostage, sem_y, sem_o):
    c = pl.program_id(0)
    RB = L // 4

    @pl.when(c == 0)
    def _():
        kv_ref[...] = jnp.zeros_like(kv_ref)
        z_ref[...] = jnp.zeros_like(z_ref)

    def bq(r):
        x = x_ref[r * 128:(r + 1) * 128, :]
        q = jnp.dot(x, wqkv_ref[:, 0:D], preferred_element_type=F32)
        pq_ref[pl.ds(pl.multiple_of(c * RB + r * 128, 128), 128), :] = _phi(q).astype(BF16)

    def bkv(r):
        x = x_ref[r * 128:(r + 1) * 128, :]
        pk = _phi(jnp.dot(x, wqkv_ref[:, D:2 * D], preferred_element_type=F32))
        z_ref[...] += jnp.sum(pk.reshape(16, 8, D), axis=0)
        pk = pk.astype(BF16)
        v = jnp.dot(x, wqkv_ref[:, 2 * D:3 * D], preferred_element_type=F32).astype(BF16)
        for t in range(4):
            sl = slice(128 * t, 128 * (t + 1))
            kv_ref[t] += lax.dot_general(pk[:, sl], v[:, sl], (((0,), (0,)), ((), ())),
                                         preferred_element_type=F32)

    def ufwd(m):
        r = jnp.dot(fu_ref[...], u_ref[m * Q:(m + 1) * Q, :], preferred_element_type=F32)
        uf[0, m] = r[:Q] + r[Q:]
        uf[1, m] = r[:Q]
        uf[2, m] = r[Q:]

    dt = jnp.exp(ldt_ref[...].astype(F32)).astype(BF16).astype(F32)
    lr = dt * are_ref[...].astype(F32)
    li = dt * aim_ref[...].astype(F32)
    e = jnp.exp(lr)
    a = (e * jnp.cos(li), e * jnp.sin(li))
    wv = _cmul((cre_ref[...].astype(F32), cim_ref[...].astype(F32)),
               (dt * bre_ref[...].astype(F32), dt * bim_ref[...].astype(F32)))
    pw = {1: a}
    p = a
    for k in range(1, 12):
        p = _csq(p)
        pw[2 ** k] = p
    p = (jnp.ones_like(lr), jnp.zeros_like(lr))
    b = wv
    for qq in range(8):
        t2r[qq * 128:(qq + 1) * 128, :] = p[0]
        t2i[qq * 128:(qq + 1) * 128, :] = p[1]
        t1r[qq * 128:(qq + 1) * 128, :] = b[0]
        t1i[qq * 128:(qq + 1) * 128, :] = b[1]
        if qq < 7:
            p = _cmul(p, a)
            b = _cmul(b, pw[128])
    for k, key in enumerate((8, 64, 1024)):
        mul_ref[2 * k] = pw[key][0]
        mul_ref[2 * k + 1] = pw[key][1]
    kl = wv[0] * pw[2048][0] - wv[1] * pw[2048][1]
    klast = jnp.sum(kl, axis=1, keepdims=True)

    def kgen(gi, _):
        for dd in range(8):
            d = gi * 8 + dd
            row = lambda k: jnp.broadcast_to(mul_ref[k, pl.ds(d, 1), :], (8, N))
            m8, m64, m1024 = (row(0), row(1)), (row(2), row(3)), (row(4), row(5))
            st = pl.ds(d, 8, stride=128)
            p = (t2r[st, :], t2i[st, :])
            rows = [p]
            for _i in range(7):
                p = _cmul(p, m8)
                rows.append(p)
            e2 = jnp.concatenate(
                [jnp.concatenate([r[0] for r in rows], 0), jnp.concatenate([r[1] for r in rows], 0)],
                1).astype(BF16)
            b0 = (t1r[st, :], t1i[st, :])
            b1 = _cmul(b0, m1024)
            b2 = _cmul(b0, m64)
            b3 = _cmul(b1, m64)
            e1 = jnp.concatenate(
                [jnp.concatenate([b0[0], b1[0], b2[0], b3[0]], 0),
                 jnp.concatenate([-b0[1], -b1[1], -b2[1], -b3[1]], 0)], 1).astype(BF16)
            res = _nt(e1, e2)
            kbuf[pl.ds(d, NC, stride=128), :] = jnp.concatenate([res[:16], res[16:]], 1)
        return 0

    for gi in range(16):
        if gi % 4 == 0:
            bq(gi // 4)
        if gi % 4 == 2:
            for m in range(gi - 2, gi + 2):
                ufwd(m)
        kgen(gi, 0)

    lane = lax.broadcasted_iota(jnp.int32, (Q, Q), 1)

    kbuf[NC * Q:(NC + 1) * Q, :] = jnp.broadcast_to(klast, (Q, Q))

    def kfwd(it, prev):
        for mm in range(4):
            m = it * 4 + mm
            kj = kbuf[pl.ds(pl.multiple_of(m * Q, Q), Q), :]
            nxt = pltpu.roll(kbuf[pl.ds(pl.multiple_of((m + 1) * Q, Q), Q), :], Q - 1, 1)
            cur = jnp.where(lane == jnp.where(m >= 2, Q - 1, -1), nxt, kj).astype(BF16)
            r = _nt(fk_ref[m], jnp.concatenate([prev, cur], 1))
            prev = cur
            kf[0, m] = r[:Q]
            kf[1, m] = r[Q:] - r[:Q]
            kf[2, m] = r[Q:] + r[:Q]
        return prev

    lax.fori_loop(0, NC // 4, kfwd, jnp.zeros((Q, Q), BF16))

    def mac(fi):
        IB = 4
        for i0 in range(0, NC, IB):
            res = []
            for h in range(2):
                fs = pl.ds(fi * 16 + h * 8, 8)
                acc = {}
                kk = {}
                for j in range(i0 + IB - 1, -1, -1):
                    uu = [uf[t, j, fs, :] for t in range(3)]
                    for i in range(i0, i0 + IB):
                        if j <= i:
                            m = i - j
                            if m not in kk:
                                kk[m] = [kf[t, m, fs, :] for t in range(3)]
                            pr = [kk[m][t] * uu[t] for t in range(3)]
                            acc[i] = pr if i not in acc else [x_ + y_ for x_, y_ in zip(acc[i], pr)]
                res.append({i: (a_[0] - a_[2], a_[0] + a_[1]) for i, a_ in acc.items()})
            for i in range(i0, i0 + IB):
                for k in range(2):
                    ybuf[i, pl.ds(k * Q + fi * 16, 16), :] = jnp.concatenate(
                        [res[0][i][k], res[1][i][k]], 0).astype(BF16)

    for fi in range(8):
        if fi % 2 == 0:
            bkv(fi // 2)
        mac(fi)

    def ycopy(cc):
        return pltpu.make_async_copy(
            ystage, out_ref.at[:, pl.ds(pl.multiple_of(cc * 128, 128), 128)], sem_y)

    @pl.when(c > 0)
    def _():
        ycopy(c - 1).wait()

    dsk = dsk_ref[...].astype(F32)
    for i in range(NC):
        y = jnp.dot(g_ref[...], ybuf[i], preferred_element_type=F32)
        ystage[i * Q:(i + 1) * Q, :] = (y + u_ref[i * Q:(i + 1) * Q, :].astype(F32) * dsk).astype(BF16)
    ycopy(c).start()

    @pl.when(c == 3)
    def _():
        r_i = lax.broadcasted_iota(jnp.int32, (128, 128), 0) // 16
        c_i = lax.broadcasted_iota(jnp.int32, (128, 128), 1) // 16
        msk = r_i == c_i
        z = jnp.sum(z_ref[...], axis=0, keepdims=True)
        zm, wc = [], []
        for t in range(4):
            sl = slice(128 * t, 128 * (t + 1))
            zt = jnp.broadcast_to(z[:, sl], (128, 128))
            zm.append(jnp.where(msk, zt, 0.0).astype(BF16))
            kvt = jnp.where(msk, kv_ref[t], 0.0).astype(BF16)
            wc.append(jnp.dot(kvt, wo_ref[sl, :], preferred_element_type=F32).astype(BF16))
        wcm = jnp.concatenate(wc, 0)
        wc_ref[...] = wcm
        for rb in range(4):
            for r in range(4):
                pq = pq_ref[rb * RB + r * 128:rb * RB + (r + 1) * 128, :]
                o = []
                for t in range(4):
                    pt = pq[:, 128 * t:128 * (t + 1)]
                    den = _nt(pt, zm[t]) + 1e-6
                    rc = pl.reciprocal(den, approx=True)
                    rc = rc * (2.0 - den * rc)
                    o.append((pt.astype(F32) * rc).astype(BF16))
                o = jnp.concatenate(o, 1)
                ostage[rb, r * 128:(r + 1) * 128, :] = jnp.dot(
                    o, wc_ref[...], preferred_element_type=F32).astype(BF16)
            pltpu.make_async_copy(ostage.at[rb], out_ref.at[rb * RB:(rb + 1) * RB, D:2 * D],
                                  sem_o.at[rb]).start()
        for rb in range(4):
            pltpu.make_async_copy(ostage.at[rb], out_ref.at[rb * RB:(rb + 1) * RB, D:2 * D],
                                  sem_o.at[rb]).wait()
        ycopy(c).wait()


@jax.jit
def pallas_concat_heads__ssm_conv_s4__linear_attn_block__prompt_kernel(
    A_u, A_A_re, A_A_im, A_B_re, A_B_im, A_C_re, A_C_im, A_log_dt, A_Dskip, B_x, B_wqkv, B_wo,
):
    par = pl.BlockSpec((128, N), lambda c: (c, 0))
    full = lambda shp: pl.BlockSpec(shp, lambda c: (0,) * len(shp))
    out = pl.pallas_call(
        _kernel,
        grid=(4,),
        in_specs=[pl.BlockSpec((L, 128), lambda c: (0, c))] + [par] * 6 + [
            pl.BlockSpec((128, 1), lambda c: (c, 0)),
            pl.BlockSpec((1, 128), lambda c: (0, c)),
            pl.BlockSpec((L // 4, D), lambda c: (c, 0)),
            full((D, 3 * D)), full((D, D)), full(_FU.shape), full(_FK.shape), full(_G.shape)],
        out_specs=pl.BlockSpec(memory_space=pl.ANY),
        out_shape=jax.ShapeDtypeStruct((L, 2 * D), BF16),
        scratch_shapes=[pltpu.VMEM((8 * 128, N), F32)] * 4 + [
            pltpu.VMEM((6, 128, N), F32),
            pltpu.VMEM(((NC + 1) * 128, Q), F32),
            pltpu.VMEM((3, NC, Q, 128), F32),
            pltpu.VMEM((3, NC, Q, 128), F32),
            pltpu.VMEM((NC, 2 * Q, 128), BF16),
            pltpu.VMEM((L, 128), BF16),
            pltpu.VMEM((L, D), BF16),
            pltpu.VMEM((4, 128, 128), F32),
            pltpu.VMEM((8, D), F32),
            pltpu.VMEM((D, D), BF16),
            pltpu.VMEM((4, L // 4, D), BF16),
            pltpu.SemaphoreType.DMA(()),
            pltpu.SemaphoreType.DMA((4,)),
        ],
        compiler_params=pltpu.CompilerParams(
            dimension_semantics=("arbitrary",), vmem_limit_bytes=100 * 1024 * 1024),
    )(A_u.reshape(L, D), A_A_re, A_A_im, A_B_re, A_B_im, A_C_re, A_C_im,
      A_log_dt.reshape(D, 1), A_Dskip.reshape(1, D), B_x.reshape(L, D), B_wqkv, B_wo,
      _FU, _FK, _G)
    return out.reshape(1, L, 2 * D)
```

```python
import jax
import jax.numpy as jnp
import numpy as np
import ml_dtypes
from jax import lax
import jax.experimental.pallas as pl
import jax.experimental.pallas.tpu as pltpu

L = 2048
D = 512
N = 128
Q = 128
NC = L // Q
F32 = jnp.float32
BF16 = jnp.bfloat16


def _consts():
    w = np.pi * (2 * np.arange(Q) + 1) / (2 * Q)
    s = np.arange(Q)
    fu = np.concatenate([np.cos(np.outer(w, s)), -np.sin(np.outer(w, s))], 0)
    g = fu.T / Q
    lr = np.arange(L).astype(np.float32).astype(ml_dtypes.bfloat16).astype(np.int64)
    fk = np.zeros((NC, 2 * Q, 2 * Q))
    for m in range(NC):
        for tau in range(-Q + 1, Q):
            l = Q * m + tau
            if l < 0:
                continue
            col = lr[l] - Q * (m - 1)
            if col == 2 * Q:
                col = 2 * Q - 1
            fk[m, :Q, col] += np.cos(w * tau)
            fk[m, Q:, col] -= np.sin(w * tau)
    b = ml_dtypes.bfloat16
    return fu.astype(b), fk.astype(b), g.astype(b)


_FU, _FK, _G = _consts()


def _cmul(a, b):
    return a[0] * b[0] - a[1] * b[1], a[0] * b[1] + a[1] * b[0]


def _csq(a):
    t = a[0] * a[1]
    return a[0] * a[0] - a[1] * a[1], t + t


def _phi(t):
    return jnp.where(t > 0, t + 1.0, jnp.exp(t)) + 1e-6


def _nt(a, b):
    return lax.dot_general(a, b, (((1,), (1,)), ((), ())), preferred_element_type=F32)


def _kernel(u_ref, are_ref, aim_ref, bre_ref, bim_ref, cre_ref, cim_ref, ldt_ref, dsk_ref,
            x_ref, wqkv_ref, wo_ref, fu_ref, fk_ref, g_ref, out_ref,
            t1r, t1i, t2r, t2i, mul_ref, kbuf, kf, uf, ybuf, ystage, pq_ref, kv_ref, z_ref,
            wc_ref, ostage, sem_y, sem_o):
    c = pl.program_id(0)
    RB = L // 4

    @pl.when(c == 0)
    def _():
        kv_ref[...] = jnp.zeros_like(kv_ref)
        z_ref[...] = jnp.zeros_like(z_ref)

    def bq(r):
        x = x_ref[r * 128:(r + 1) * 128, :]
        q = jnp.dot(x, wqkv_ref[:, 0:D], preferred_element_type=F32)
        pq_ref[pl.ds(pl.multiple_of(c * RB + r * 128, 128), 128), :] = _phi(q).astype(BF16)

    def bkv_pieces():
        for r in range(4):
            for hh in range(2):
                x = x_ref[r * 128:(r + 1) * 128, :]
                cs = slice(256 * hh, 256 * (hh + 1))
                pk = _phi(jnp.dot(x, wqkv_ref[:, D + 256 * hh:D + 256 * (hh + 1)],
                                  preferred_element_type=F32))
                z_ref[:, cs] += jnp.sum(pk.reshape(16, 8, 256), axis=0)
                pk = pk.astype(BF16)
                yield
                v = jnp.dot(x, wqkv_ref[:, 2 * D + 256 * hh:2 * D + 256 * (hh + 1)],
                            preferred_element_type=F32).astype(BF16)
                yield
                for t in range(2):
                    sl = slice(128 * t, 128 * (t + 1))
                    kv_ref[2 * hh + t] += lax.dot_general(
                        pk[:, sl], v[:, sl], (((0,), (0,)), ((), ())), preferred_element_type=F32)
                    yield

    bgen = bkv_pieces()

    def ufwd(m):
        r = jnp.dot(fu_ref[...], u_ref[m * Q:(m + 1) * Q, :], preferred_element_type=F32)
        uf[0, m] = r[:Q] + r[Q:]
        uf[1, m] = r[:Q]
        uf[2, m] = r[Q:]

    dt = jnp.exp(ldt_ref[...].astype(F32)).astype(BF16).astype(F32)
    lr = dt * are_ref[...].astype(F32)
    li = dt * aim_ref[...].astype(F32)
    e = jnp.exp(lr)
    a = (e * jnp.cos(li), e * jnp.sin(li))
    wv = _cmul((cre_ref[...].astype(F32), cim_ref[...].astype(F32)),
               (dt * bre_ref[...].astype(F32), dt * bim_ref[...].astype(F32)))
    pw = {1: a}
    p = a
    for k in range(1, 12):
        p = _csq(p)
        pw[2 ** k] = p
    p = (jnp.ones_like(lr), jnp.zeros_like(lr))
    b = wv
    for qq in range(8):
        t2r[qq * 128:(qq + 1) * 128, :] = p[0]
        t2i[qq * 128:(qq + 1) * 128, :] = p[1]
        t1r[qq * 128:(qq + 1) * 128, :] = b[0]
        t1i[qq * 128:(qq + 1) * 128, :] = b[1]
        if qq < 7:
            p = _cmul(p, a)
            b = _cmul(b, pw[128])
    for k, key in enumerate((8, 64, 1024)):
        mul_ref[2 * k] = pw[key][0]
        mul_ref[2 * k + 1] = pw[key][1]
    kl = wv[0] * pw[2048][0] - wv[1] * pw[2048][1]
    klast = jnp.sum(kl, axis=1, keepdims=True)

    def kgen(gi, _):
        for dd in range(8):
            d = gi * 8 + dd
            row = lambda k: jnp.broadcast_to(mul_ref[k, pl.ds(d, 1), :], (8, N))
            m8, m64, m1024 = (row(0), row(1)), (row(2), row(3)), (row(4), row(5))
            st = pl.ds(d, 8, stride=128)
            p = (t2r[st, :], t2i[st, :])
            rows = [p]
            for _i in range(7):
                p = _cmul(p, m8)
                rows.append(p)
            e2 = jnp.concatenate(
                [jnp.concatenate([r[0] for r in rows], 0), jnp.concatenate([r[1] for r in rows], 0)],
                1).astype(BF16)
            b0 = (t1r[st, :], t1i[st, :])
            b1 = _cmul(b0, m1024)
            b2 = _cmul(b0, m64)
            b3 = _cmul(b1, m64)
            e1 = jnp.concatenate(
                [jnp.concatenate([b0[0], b1[0], b2[0], b3[0]], 0),
                 jnp.concatenate([-b0[1], -b1[1], -b2[1], -b3[1]], 0)], 1).astype(BF16)
            res = _nt(e1, e2)
            kbuf[pl.ds(d, NC, stride=128), :] = jnp.concatenate([res[:16], res[16:]], 1)
        return 0

    for gi in range(16):
        if gi % 4 == 0:
            bq(gi // 4)
        if gi % 4 == 2:
            for m in range(gi - 2, gi + 2):
                ufwd(m)
        kgen(gi, 0)

    lane = lax.broadcasted_iota(jnp.int32, (Q, Q), 1)

    kbuf[NC * Q:(NC + 1) * Q, :] = jnp.broadcast_to(klast, (Q, Q))

    def kfwd(it, prev):
        for mm in range(4):
            m = it * 4 + mm
            kj = kbuf[pl.ds(pl.multiple_of(m * Q, Q), Q), :]
            nxt = pltpu.roll(kbuf[pl.ds(pl.multiple_of((m + 1) * Q, Q), Q), :], Q - 1, 1)
            cur = jnp.where(lane == jnp.where(m >= 2, Q - 1, -1), nxt, kj).astype(BF16)
            r = _nt(fk_ref[m], jnp.concatenate([prev, cur], 1))
            prev = cur
            kf[0, m] = r[:Q]
            kf[1, m] = r[Q:] - r[:Q]
            kf[2, m] = r[Q:] + r[:Q]
        return prev

    lax.fori_loop(0, NC // 4, kfwd, jnp.zeros((Q, Q), BF16))

    def mac(fi):
        IB = 4
        for i0 in range(0, NC, IB):
            next(bgen, None)
            res = []
            for h in range(2):
                fs = pl.ds(fi * 16 + h * 8, 8)
                acc = {}
                kk = {}
                for j in range(i0 + IB - 1, -1, -1):
                    uu = [uf[t, j, fs, :] for t in range(3)]
                    for i in range(i0, i0 + IB):
                        if j <= i:
                            m = i - j
                            if m not in kk:
                                kk[m] = [kf[t, m, fs, :] for t in range(3)]
                            pr = [kk[m][t] * uu[t] for t in range(3)]
                            acc[i] = pr if i not in acc else [x_ + y_ for x_, y_ in zip(acc[i], pr)]
                res.append({i: (a_[0] - a_[2], a_[0] + a_[1]) for i, a_ in acc.items()})
            for i in range(i0, i0 + IB):
                for k in range(2):
                    ybuf[i, pl.ds(k * Q + fi * 16, 16), :] = jnp.concatenate(
                        [res[0][i][k], res[1][i][k]], 0).astype(BF16)

    for fi in range(8):
        mac(fi)

    def ycopy(cc):
        return pltpu.make_async_copy(
            ystage, out_ref.at[:, pl.ds(pl.multiple_of(cc * 128, 128), 128)], sem_y)

    @pl.when(c > 0)
    def _():
        ycopy(c - 1).wait()

    dsk = dsk_ref[...].astype(F32)
    for i in range(NC):
        y = jnp.dot(g_ref[...], ybuf[i], preferred_element_type=F32)
        ystage[i * Q:(i + 1) * Q, :] = (y + u_ref[i * Q:(i + 1) * Q, :].astype(F32) * dsk).astype(BF16)
    ycopy(c).start()

    @pl.when(c == 3)
    def _():
        r_i = lax.broadcasted_iota(jnp.int32, (128, 128), 0) // 16
        c_i = lax.broadcasted_iota(jnp.int32, (128, 128), 1) // 16
        msk = r_i == c_i
        z = jnp.sum(z_ref[...], axis=0, keepdims=True)
        zm, wc = [], []
        for t in range(4):
            sl = slice(128 * t, 128 * (t + 1))
            zt = jnp.broadcast_to(z[:, sl], (128, 128))
            zm.append(jnp.where(msk, zt, 0.0).astype(BF16))
            kvt = jnp.where(msk, kv_ref[t], 0.0).astype(BF16)
            wc.append(jnp.dot(kvt, wo_ref[sl, :], preferred_element_type=F32).astype(BF16))
        wcm = jnp.concatenate(wc, 0)
        wc_ref[...] = wcm
        for rb in range(4):
            for r in range(4):
                pq = pq_ref[rb * RB + r * 128:rb * RB + (r + 1) * 128, :]
                o = []
                for t in range(4):
                    pt = pq[:, 128 * t:128 * (t + 1)]
                    den = _nt(pt, zm[t]) + 1e-6
                    rc = pl.reciprocal(den, approx=True)
                    rc = rc * (2.0 - den * rc)
                    o.append((pt.astype(F32) * rc).astype(BF16))
                o = jnp.concatenate(o, 1)
                ostage[rb, r * 128:(r + 1) * 128, :] = jnp.dot(
                    o, wc_ref[...], preferred_element_type=F32).astype(BF16)
            pltpu.make_async_copy(ostage.at[rb], out_ref.at[rb * RB:(rb + 1) * RB, D:2 * D],
                                  sem_o.at[rb]).start()
        for rb in range(4):
            pltpu.make_async_copy(ostage.at[rb], out_ref.at[rb * RB:(rb + 1) * RB, D:2 * D],
                                  sem_o.at[rb]).wait()
        ycopy(c).wait()


@jax.jit
def pallas_concat_heads__ssm_conv_s4__linear_attn_block__prompt_kernel(
    A_u, A_A_re, A_A_im, A_B_re, A_B_im, A_C_re, A_C_im, A_log_dt, A_Dskip, B_x, B_wqkv, B_wo,
):
    par = pl.BlockSpec((128, N), lambda c: (c, 0))
    full = lambda shp: pl.BlockSpec(shp, lambda c: (0,) * len(shp))
    out = pl.pallas_call(
        _kernel,
        grid=(4,),
        in_specs=[pl.BlockSpec((L, 128), lambda c: (0, c))] + [par] * 6 + [
            pl.BlockSpec((128, 1), lambda c: (c, 0)),
            pl.BlockSpec((1, 128), lambda c: (0, c)),
            pl.BlockSpec((L // 4, D), lambda c: (c, 0)),
            full((D, 3 * D)), full((D, D)), full(_FU.shape), full(_FK.shape), full(_G.shape)],
        out_specs=pl.BlockSpec(memory_space=pl.ANY),
        out_shape=jax.ShapeDtypeStruct((L, 2 * D), BF16),
        scratch_shapes=[pltpu.VMEM((8 * 128, N), F32)] * 4 + [
            pltpu.VMEM((6, 128, N), F32),
            pltpu.VMEM(((NC + 1) * 128, Q), F32),
            pltpu.VMEM((3, NC, Q, 128), F32),
            pltpu.VMEM((3, NC, Q, 128), F32),
            pltpu.VMEM((NC, 2 * Q, 128), BF16),
            pltpu.VMEM((L, 128), BF16),
            pltpu.VMEM((L, D), BF16),
            pltpu.VMEM((4, 128, 128), F32),
            pltpu.VMEM((8, D), F32),
            pltpu.VMEM((D, D), BF16),
            pltpu.VMEM((4, L // 4, D), BF16),
            pltpu.SemaphoreType.DMA(()),
            pltpu.SemaphoreType.DMA((4,)),
        ],
        compiler_params=pltpu.CompilerParams(
            dimension_semantics=("arbitrary",), vmem_limit_bytes=100 * 1024 * 1024),
    )(A_u.reshape(L, D), A_A_re, A_A_im, A_B_re, A_B_im, A_C_re, A_C_im,
      A_log_dt.reshape(D, 1), A_Dskip.reshape(1, D), B_x.reshape(L, D), B_wqkv, B_wo,
      _FU, _FK, _G)
    return out.reshape(1, L, 2 * D)
```

```python
import jax
import jax.numpy as jnp
import numpy as np
import ml_dtypes
from jax import lax
import jax.experimental.pallas as pl
import jax.experimental.pallas.tpu as pltpu

L = 2048
D = 512
N = 128
Q = 128
NC = L // Q
F32 = jnp.float32
BF16 = jnp.bfloat16


def _consts():
    w = np.pi * (2 * np.arange(Q) + 1) / (2 * Q)
    s = np.arange(Q)
    fu = np.concatenate([np.cos(np.outer(w, s)), -np.sin(np.outer(w, s))], 0)
    g = fu.T / Q
    lr = np.arange(L).astype(np.float32).astype(ml_dtypes.bfloat16).astype(np.int64)
    fk = np.zeros((NC, 2 * Q, 2 * Q))
    for m in range(NC):
        for tau in range(-Q + 1, Q):
            l = Q * m + tau
            if l < 0:
                continue
            col = lr[l] - Q * (m - 1)
            if col == 2 * Q:
                col = 2 * Q - 1
            fk[m, :Q, col] += np.cos(w * tau)
            fk[m, Q:, col] -= np.sin(w * tau)
    b = ml_dtypes.bfloat16
    return fu.astype(b), fk.astype(b), g.astype(b)


_FU, _FK, _G = _consts()


def _cmul(a, b):
    return a[0] * b[0] - a[1] * b[1], a[0] * b[1] + a[1] * b[0]


def _csq(a):
    t = a[0] * a[1]
    return a[0] * a[0] - a[1] * a[1], t + t


def _phi(t):
    return jnp.where(t > 0, t + 1.0, jnp.exp(t)) + 1e-6


def _nt(a, b):
    return lax.dot_general(a, b, (((1,), (1,)), ((), ())), preferred_element_type=F32)


def _kernel(u_ref, are_ref, aim_ref, bre_ref, bim_ref, cre_ref, cim_ref, ldt_ref, dsk_ref,
            x_ref, wqkv_ref, wo_ref, fu_ref, fk_ref, g_ref, out_ref,
            t1r, t1i, t2r, t2i, mul_ref, kbuf, kf, uf, ybuf, ystage, pq_ref, kv_ref, z_ref,
            wc_ref, ostage, sem_y, sem_o):
    c = pl.program_id(0)
    RB = L // 4

    @pl.when(c == 0)
    def _():
        kv_ref[...] = jnp.zeros_like(kv_ref)
        z_ref[...] = jnp.zeros_like(z_ref)

    def bq(r):
        x = x_ref[r * 128:(r + 1) * 128, :]
        q = jnp.dot(x, wqkv_ref[:, 0:D], preferred_element_type=F32)
        pq_ref[pl.ds(pl.multiple_of(c * RB + r * 128, 128), 128), :] = _phi(q).astype(BF16)

    zacc, kvacc = {}, {}

    def bkv_pieces():
        for r in range(4):
            for hh in range(2):
                x = x_ref[r * 128:(r + 1) * 128, :]
                cs = slice(256 * hh, 256 * (hh + 1))
                pk = _phi(jnp.dot(x, wqkv_ref[:, D + 256 * hh:D + 256 * (hh + 1)],
                                  preferred_element_type=F32))
                zacc[hh] = zacc.get(hh, 0.0) + jnp.sum(pk.reshape(16, 8, 256), axis=0)
                pk = pk.astype(BF16)
                yield
                v = jnp.dot(x, wqkv_ref[:, 2 * D + 256 * hh:2 * D + 256 * (hh + 1)],
                            preferred_element_type=F32).astype(BF16)
                yield
                for t in range(2):
                    sl = slice(128 * t, 128 * (t + 1))
                    kvacc[2 * hh + t] = kvacc.get(2 * hh + t, 0.0) + lax.dot_general(
                        pk[:, sl], v[:, sl], (((0,), (0,)), ((), ())), preferred_element_type=F32)
                    yield

    bgen = bkv_pieces()

    def ufwd(m):
        r = jnp.dot(fu_ref[...], u_ref[m * Q:(m + 1) * Q, :], preferred_element_type=F32)
        uf[0, m] = r[:Q] + r[Q:]
        uf[1, m] = r[:Q]
        uf[2, m] = r[Q:]

    dt = jnp.exp(ldt_ref[...].astype(F32)).astype(BF16).astype(F32)
    lr = dt * are_ref[...].astype(F32)
    li = dt * aim_ref[...].astype(F32)
    e = jnp.exp(lr)
    a = (e * jnp.cos(li), e * jnp.sin(li))
    wv = _cmul((cre_ref[...].astype(F32), cim_ref[...].astype(F32)),
               (dt * bre_ref[...].astype(F32), dt * bim_ref[...].astype(F32)))
    pw = {1: a}
    p = a
    for k in range(1, 12):
        p = _csq(p)
        pw[2 ** k] = p
    p = (jnp.ones_like(lr), jnp.zeros_like(lr))
    b = wv
    for qq in range(8):
        t2r[qq * 128:(qq + 1) * 128, :] = p[0]
        t2i[qq * 128:(qq + 1) * 128, :] = p[1]
        t1r[qq * 128:(qq + 1) * 128, :] = b[0]
        t1i[qq * 128:(qq + 1) * 128, :] = b[1]
        if qq < 7:
            p = _cmul(p, a)
            b = _cmul(b, pw[128])
    for k, key in enumerate((8, 64, 1024)):
        mul_ref[2 * k] = pw[key][0]
        mul_ref[2 * k + 1] = pw[key][1]
    kl = wv[0] * pw[2048][0] - wv[1] * pw[2048][1]
    klast = jnp.sum(kl, axis=1, keepdims=True)

    def kgen(gi, _):
        for dd in range(8):
            if dd % 4 == 0:
                next(bgen, None)
            d = gi * 8 + dd
            row = lambda k: jnp.broadcast_to(mul_ref[k, pl.ds(d, 1), :], (8, N))
            m8, m64, m1024 = (row(0), row(1)), (row(2), row(3)), (row(4), row(5))
            st = pl.ds(d, 8, stride=128)
            p = (t2r[st, :], t2i[st, :])
            rows = [p]
            for _i in range(7):
                p = _cmul(p, m8)
                rows.append(p)
            e2 = jnp.concatenate(
                [jnp.concatenate([r[0] for r in rows], 0), jnp.concatenate([r[1] for r in rows], 0)],
                1).astype(BF16)
            b0 = (t1r[st, :], t1i[st, :])
            b1 = _cmul(b0, m1024)
            b2 = _cmul(b0, m64)
            b3 = _cmul(b1, m64)
            e1 = jnp.concatenate(
                [jnp.concatenate([b0[0], b1[0], b2[0], b3[0]], 0),
                 jnp.concatenate([-b0[1], -b1[1], -b2[1], -b3[1]], 0)], 1).astype(BF16)
            res = _nt(e1, e2)
            kbuf[pl.ds(d, NC, stride=128), :] = jnp.concatenate([res[:16], res[16:]], 1)
        return 0

    for gi in range(16):
        if gi % 4 == 0:
            bq(gi // 4)
        if gi % 4 == 2:
            for m in range(gi - 2, gi + 2):
                ufwd(m)
        kgen(gi, 0)

    lane = lax.broadcasted_iota(jnp.int32, (Q, Q), 1)

    kbuf[NC * Q:(NC + 1) * Q, :] = jnp.broadcast_to(klast, (Q, Q))

    def kfwd(it, prev):
        for mm in range(4):
            m = it * 4 + mm
            kj = kbuf[pl.ds(pl.multiple_of(m * Q, Q), Q), :]
            nxt = pltpu.roll(kbuf[pl.ds(pl.multiple_of((m + 1) * Q, Q), Q), :], Q - 1, 1)
            cur = jnp.where(lane == jnp.where(m >= 2, Q - 1, -1), nxt, kj).astype(BF16)
            r = _nt(fk_ref[m], jnp.concatenate([prev, cur], 1))
            prev = cur
            kf[0, m] = r[:Q]
            kf[1, m] = r[Q:] - r[:Q]
            kf[2, m] = r[Q:] + r[:Q]
        return prev

    lax.fori_loop(0, NC // 4, kfwd, jnp.zeros((Q, Q), BF16))

    def mac(fi):
        IB = 4
        for i0 in range(0, NC, IB):
            res = []
            for h in range(2):
                fs = pl.ds(fi * 16 + h * 8, 8)
                acc = {}
                kk = {}
                for j in range(i0 + IB - 1, -1, -1):
                    uu = [uf[t, j, fs, :] for t in range(3)]
                    for i in range(i0, i0 + IB):
                        if j <= i:
                            m = i - j
                            if m not in kk:
                                kk[m] = [kf[t, m, fs, :] for t in range(3)]
                            pr = [kk[m][t] * uu[t] for t in range(3)]
                            acc[i] = pr if i not in acc else [x_ + y_ for x_, y_ in zip(acc[i], pr)]
                res.append({i: (a_[0] - a_[2], a_[0] + a_[1]) for i, a_ in acc.items()})
            for i in range(i0, i0 + IB):
                for k in range(2):
                    ybuf[i, pl.ds(k * Q + fi * 16, 16), :] = jnp.concatenate(
                        [res[0][i][k], res[1][i][k]], 0).astype(BF16)

    for fi in range(8):
        mac(fi)
    for hh in range(2):
        z_ref[:, 256 * hh:256 * (hh + 1)] += zacc[hh]
    for t in range(4):
        kv_ref[t] += kvacc[t]

    def ycopy(cc):
        return pltpu.make_async_copy(
            ystage, out_ref.at[:, pl.ds(pl.multiple_of(cc * 128, 128), 128)], sem_y)

    @pl.when(c > 0)
    def _():
        ycopy(c - 1).wait()

    dsk = dsk_ref[...].astype(F32)
    for i in range(NC):
        y = jnp.dot(g_ref[...], ybuf[i], preferred_element_type=F32)
        ystage[i * Q:(i + 1) * Q, :] = (y + u_ref[i * Q:(i + 1) * Q, :].astype(F32) * dsk).astype(BF16)
    ycopy(c).start()

    @pl.when(c == 3)
    def _():
        r_i = lax.broadcasted_iota(jnp.int32, (128, 128), 0) // 16
        c_i = lax.broadcasted_iota(jnp.int32, (128, 128), 1) // 16
        msk = r_i == c_i
        z = jnp.sum(z_ref[...], axis=0, keepdims=True)
        zm, wc = [], []
        for t in range(4):
            sl = slice(128 * t, 128 * (t + 1))
            zt = jnp.broadcast_to(z[:, sl], (128, 128))
            zm.append(jnp.where(msk, zt, 0.0).astype(BF16))
            kvt = jnp.where(msk, kv_ref[t], 0.0).astype(BF16)
            wc.append(jnp.dot(kvt, wo_ref[sl, :], preferred_element_type=F32).astype(BF16))
        wcm = jnp.concatenate(wc, 0)
        wc_ref[...] = wcm
        for rb in range(4):
            for r in range(4):
                pq = pq_ref[rb * RB + r * 128:rb * RB + (r + 1) * 128, :]
                o = []
                for t in range(4):
                    pt = pq[:, 128 * t:128 * (t + 1)]
                    den = _nt(pt, zm[t]) + 1e-6
                    rc = pl.reciprocal(den, approx=True)
                    rc = rc * (2.0 - den * rc)
                    o.append((pt.astype(F32) * rc).astype(BF16))
                o = jnp.concatenate(o, 1)
                ostage[rb, r * 128:(r + 1) * 128, :] = jnp.dot(
                    o, wc_ref[...], preferred_element_type=F32).astype(BF16)
            pltpu.make_async_copy(ostage.at[rb], out_ref.at[rb * RB:(rb + 1) * RB, D:2 * D],
                                  sem_o.at[rb]).start()
        for rb in range(4):
            pltpu.make_async_copy(ostage.at[rb], out_ref.at[rb * RB:(rb + 1) * RB, D:2 * D],
                                  sem_o.at[rb]).wait()
        ycopy(c).wait()


@jax.jit
def pallas_concat_heads__ssm_conv_s4__linear_attn_block__prompt_kernel(
    A_u, A_A_re, A_A_im, A_B_re, A_B_im, A_C_re, A_C_im, A_log_dt, A_Dskip, B_x, B_wqkv, B_wo,
):
    par = pl.BlockSpec((128, N), lambda c: (c, 0))
    full = lambda shp: pl.BlockSpec(shp, lambda c: (0,) * len(shp))
    out = pl.pallas_call(
        _kernel,
        grid=(4,),
        in_specs=[pl.BlockSpec((L, 128), lambda c: (0, c))] + [par] * 6 + [
            pl.BlockSpec((128, 1), lambda c: (c, 0)),
            pl.BlockSpec((1, 128), lambda c: (0, c)),
            pl.BlockSpec((L // 4, D), lambda c: (c, 0)),
            full((D, 3 * D)), full((D, D)), full(_FU.shape), full(_FK.shape), full(_G.shape)],
        out_specs=pl.BlockSpec(memory_space=pl.ANY),
        out_shape=jax.ShapeDtypeStruct((L, 2 * D), BF16),
        scratch_shapes=[pltpu.VMEM((8 * 128, N), F32)] * 4 + [
            pltpu.VMEM((6, 128, N), F32),
            pltpu.VMEM(((NC + 1) * 128, Q), F32),
            pltpu.VMEM((3, NC, Q, 128), F32),
            pltpu.VMEM((3, NC, Q, 128), F32),
            pltpu.VMEM((NC, 2 * Q, 128), BF16),
            pltpu.VMEM((L, 128), BF16),
            pltpu.VMEM((L, D), BF16),
            pltpu.VMEM((4, 128, 128), F32),
            pltpu.VMEM((8, D), F32),
            pltpu.VMEM((D, D), BF16),
            pltpu.VMEM((4, L // 4, D), BF16),
            pltpu.SemaphoreType.DMA(()),
            pltpu.SemaphoreType.DMA((4,)),
        ],
        compiler_params=pltpu.CompilerParams(
            dimension_semantics=("arbitrary",), vmem_limit_bytes=100 * 1024 * 1024),
    )(A_u.reshape(L, D), A_A_re, A_A_im, A_B_re, A_B_im, A_C_re, A_C_im,
      A_log_dt.reshape(D, 1), A_Dskip.reshape(1, D), B_x.reshape(L, D), B_wqkv, B_wo,
      _FU, _FK, _G)
    return out.reshape(1, L, 2 * D)
```

```python
import jax
import jax.numpy as jnp
import numpy as np
import ml_dtypes
from jax import lax
import jax.experimental.pallas as pl
import jax.experimental.pallas.tpu as pltpu

L = 2048
D = 512
N = 128
Q = 128
NC = L // Q
F32 = jnp.float32
BF16 = jnp.bfloat16


def _consts():
    w = np.pi * (2 * np.arange(Q) + 1) / (2 * Q)
    s = np.arange(Q)
    fu = np.concatenate([np.cos(np.outer(w, s)), -np.sin(np.outer(w, s))], 0)
    g = fu.T / Q
    lr = np.arange(L).astype(np.float32).astype(ml_dtypes.bfloat16).astype(np.int64)
    fk = np.zeros((NC, 2 * Q, 2 * Q))
    for m in range(NC):
        for tau in range(-Q + 1, Q):
            l = Q * m + tau
            if l < 0:
                continue
            col = lr[l] - Q * (m - 1)
            if col == 2 * Q:
                col = 2 * Q - 1
            fk[m, :Q, col] += np.cos(w * tau)
            fk[m, Q:, col] -= np.sin(w * tau)
    b = ml_dtypes.bfloat16
    return fu.astype(b), fk.astype(b), g.astype(b)


_FU, _FK, _G = _consts()


def _cmul(a, b):
    return a[0] * b[0] - a[1] * b[1], a[0] * b[1] + a[1] * b[0]


def _csq(a):
    t = a[0] * a[1]
    return a[0] * a[0] - a[1] * a[1], t + t


def _phi(t):
    return jnp.where(t > 0, t + 1.0, jnp.exp(t)) + 1e-6


def _nt(a, b):
    return lax.dot_general(a, b, (((1,), (1,)), ((), ())), preferred_element_type=F32)


def _kernel(u_ref, are_ref, aim_ref, bre_ref, bim_ref, cre_ref, cim_ref, ldt_ref, dsk_ref,
            x_ref, wqkv_ref, wo_ref, fu_ref, fk_ref, g_ref, out_ref,
            t1r, t1i, t2r, t2i, mul_ref, kbuf, kf, uf, ybuf, ystage, pq_ref, kv_ref, z_ref,
            wc_ref, ostage, sem_y, sem_o):
    c = pl.program_id(0)
    RB = L // 4

    @pl.when(c == 0)
    def _():
        kv_ref[...] = jnp.zeros_like(kv_ref)
        z_ref[...] = jnp.zeros_like(z_ref)

    def bq(r):
        x = x_ref[r * 128:(r + 1) * 128, :]
        q = jnp.dot(x, wqkv_ref[:, 0:D], preferred_element_type=F32)
        pq_ref[pl.ds(pl.multiple_of(c * RB + r * 128, 128), 128), :] = _phi(q).astype(BF16)

    zacc, kvacc = {}, {}

    def bkv_pieces():
        for r in range(4):
            for hh in range(1):
                x = x_ref[r * 128:(r + 1) * 128, :]
                cs = slice(512 * hh, 512 * (hh + 1))
                pk = _phi(jnp.dot(x, wqkv_ref[:, D + 512 * hh:D + 512 * (hh + 1)],
                                  preferred_element_type=F32))
                zacc[hh] = zacc.get(hh, 0.0) + jnp.sum(pk.reshape(16, 8, 512), axis=0)
                pk = pk.astype(BF16)
                yield
                v = jnp.dot(x, wqkv_ref[:, 2 * D + 512 * hh:2 * D + 512 * (hh + 1)],
                            preferred_element_type=F32).astype(BF16)
                yield
                for t in range(4):
                    sl = slice(128 * t, 128 * (t + 1))
                    kvacc[2 * hh + t] = kvacc.get(2 * hh + t, 0.0) + lax.dot_general(
                        pk[:, sl], v[:, sl], (((0,), (0,)), ((), ())), preferred_element_type=F32)
                    yield

    bgen = bkv_pieces()

    def ufwd(m):
        r = jnp.dot(fu_ref[...], u_ref[m * Q:(m + 1) * Q, :], preferred_element_type=F32)
        uf[0, m] = r[:Q] + r[Q:]
        uf[1, m] = r[:Q]
        uf[2, m] = r[Q:]

    dt = jnp.exp(ldt_ref[...].astype(F32)).astype(BF16).astype(F32)
    lr = dt * are_ref[...].astype(F32)
    li = dt * aim_ref[...].astype(F32)
    e = jnp.exp(lr)
    a = (e * jnp.cos(li), e * jnp.sin(li))
    wv = _cmul((cre_ref[...].astype(F32), cim_ref[...].astype(F32)),
               (dt * bre_ref[...].astype(F32), dt * bim_ref[...].astype(F32)))
    pw = {1: a}
    p = a
    for k in range(1, 12):
        p = _csq(p)
        pw[2 ** k] = p
    p = (jnp.ones_like(lr), jnp.zeros_like(lr))
    b = wv
    for qq in range(8):
        t2r[qq * 128:(qq + 1) * 128, :] = p[0]
        t2i[qq * 128:(qq + 1) * 128, :] = p[1]
        t1r[qq * 128:(qq + 1) * 128, :] = b[0]
        t1i[qq * 128:(qq + 1) * 128, :] = b[1]
        if qq < 7:
            p = _cmul(p, a)
            b = _cmul(b, pw[128])
    for k, key in enumerate((8, 64, 1024)):
        mul_ref[2 * k] = pw[key][0]
        mul_ref[2 * k + 1] = pw[key][1]
    kl = wv[0] * pw[2048][0] - wv[1] * pw[2048][1]
    klast = jnp.sum(kl, axis=1, keepdims=True)

    def kgen(gi, _):
        for dd in range(8):
            if dd % 4 == 0:
                next(bgen, None)
            d = gi * 8 + dd
            row = lambda k: jnp.broadcast_to(mul_ref[k, pl.ds(d, 1), :], (8, N))
            m8, m64, m1024 = (row(0), row(1)), (row(2), row(3)), (row(4), row(5))
            st = pl.ds(d, 8, stride=128)
            p = (t2r[st, :], t2i[st, :])
            rows = [p]
            for _i in range(7):
                p = _cmul(p, m8)
                rows.append(p)
            e2 = jnp.concatenate(
                [jnp.concatenate([r[0] for r in rows], 0), jnp.concatenate([r[1] for r in rows], 0)],
                1).astype(BF16)
            b0 = (t1r[st, :], t1i[st, :])
            b1 = _cmul(b0, m1024)
            b2 = _cmul(b0, m64)
            b3 = _cmul(b1, m64)
            e1 = jnp.concatenate(
                [jnp.concatenate([b0[0], b1[0], b2[0], b3[0]], 0),
                 jnp.concatenate([-b0[1], -b1[1], -b2[1], -b3[1]], 0)], 1).astype(BF16)
            res = _nt(e1, e2)
            kbuf[pl.ds(d, NC, stride=128), :] = jnp.concatenate([res[:16], res[16:]], 1)
        return 0

    for gi in range(16):
        if gi % 4 == 0:
            bq(gi // 4)
        if gi % 4 == 2:
            for m in range(gi - 2, gi + 2):
                ufwd(m)
        kgen(gi, 0)

    lane = lax.broadcasted_iota(jnp.int32, (Q, Q), 1)

    kbuf[NC * Q:(NC + 1) * Q, :] = jnp.broadcast_to(klast, (Q, Q))

    def kfwd(it, prev):
        for mm in range(4):
            m = it * 4 + mm
            kj = kbuf[pl.ds(pl.multiple_of(m * Q, Q), Q), :]
            nxt = pltpu.roll(kbuf[pl.ds(pl.multiple_of((m + 1) * Q, Q), Q), :], Q - 1, 1)
            cur = jnp.where(lane == jnp.where(m >= 2, Q - 1, -1), nxt, kj).astype(BF16)
            r = _nt(fk_ref[m], jnp.concatenate([prev, cur], 1))
            prev = cur
            kf[0, m] = r[:Q]
            kf[1, m] = r[Q:] - r[:Q]
            kf[2, m] = r[Q:] + r[:Q]
        return prev

    lax.fori_loop(0, NC // 4, kfwd, jnp.zeros((Q, Q), BF16))

    def mac(fi):
        IB = 4
        for i0 in range(0, NC, IB):
            res = []
            for h in range(2):
                fs = pl.ds(fi * 16 + h * 8, 8)
                acc = {}
                kk = {}
                for j in range(i0 + IB - 1, -1, -1):
                    uu = [uf[t, j, fs, :] for t in range(3)]
                    for i in range(i0, i0 + IB):
                        if j <= i:
                            m = i - j
                            if m not in kk:
                                kk[m] = [kf[t, m, fs, :] for t in range(3)]
                            pr = [kk[m][t] * uu[t] for t in range(3)]
                            acc[i] = pr if i not in acc else [x_ + y_ for x_, y_ in zip(acc[i], pr)]
                res.append({i: (a_[0] - a_[2], a_[0] + a_[1]) for i, a_ in acc.items()})
            for i in range(i0, i0 + IB):
                for k in range(2):
                    ybuf[i, pl.ds(k * Q + fi * 16, 16), :] = jnp.concatenate(
                        [res[0][i][k], res[1][i][k]], 0).astype(BF16)

    for fi in range(8):
        mac(fi)
    for hh in range(1):
        z_ref[:, 512 * hh:512 * (hh + 1)] += zacc[hh]
    for t in range(4):
        kv_ref[t] += kvacc[t]

    def ycopy(cc):
        return pltpu.make_async_copy(
            ystage, out_ref.at[:, pl.ds(pl.multiple_of(cc * 128, 128), 128)], sem_y)

    @pl.when(c > 0)
    def _():
        ycopy(c - 1).wait()

    dsk = dsk_ref[...].astype(F32)
    for i in range(NC):
        y = jnp.dot(g_ref[...], ybuf[i], preferred_element_type=F32)
        ystage[i * Q:(i + 1) * Q, :] = (y + u_ref[i * Q:(i + 1) * Q, :].astype(F32) * dsk).astype(BF16)
    ycopy(c).start()

    @pl.when(c == 3)
    def _():
        r_i = lax.broadcasted_iota(jnp.int32, (128, 128), 0) // 16
        c_i = lax.broadcasted_iota(jnp.int32, (128, 128), 1) // 16
        msk = r_i == c_i
        z = jnp.sum(z_ref[...], axis=0, keepdims=True)
        zm, wc = [], []
        for t in range(4):
            sl = slice(128 * t, 128 * (t + 1))
            zt = jnp.broadcast_to(z[:, sl], (128, 128))
            zm.append(jnp.where(msk, zt, 0.0).astype(BF16))
            kvt = jnp.where(msk, kv_ref[t], 0.0).astype(BF16)
            wc.append(jnp.dot(kvt, wo_ref[sl, :], preferred_element_type=F32).astype(BF16))
        wcm = jnp.concatenate(wc, 0)
        wc_ref[...] = wcm
        for rb in range(4):
            for r in range(4):
                pq = pq_ref[rb * RB + r * 128:rb * RB + (r + 1) * 128, :]
                o = []
                for t in range(4):
                    pt = pq[:, 128 * t:128 * (t + 1)]
                    den = _nt(pt, zm[t]) + 1e-6
                    rc = pl.reciprocal(den, approx=True)
                    rc = rc * (2.0 - den * rc)
                    o.append((pt.astype(F32) * rc).astype(BF16))
                o = jnp.concatenate(o, 1)
                ostage[rb, r * 128:(r + 1) * 128, :] = jnp.dot(
                    o, wc_ref[...], preferred_element_type=F32).astype(BF16)
            pltpu.make_async_copy(ostage.at[rb], out_ref.at[rb * RB:(rb + 1) * RB, D:2 * D],
                                  sem_o.at[rb]).start()
        for rb in range(4):
            pltpu.make_async_copy(ostage.at[rb], out_ref.at[rb * RB:(rb + 1) * RB, D:2 * D],
                                  sem_o.at[rb]).wait()
        ycopy(c).wait()


@jax.jit
def pallas_concat_heads__ssm_conv_s4__linear_attn_block__prompt_kernel(
    A_u, A_A_re, A_A_im, A_B_re, A_B_im, A_C_re, A_C_im, A_log_dt, A_Dskip, B_x, B_wqkv, B_wo,
):
    par = pl.BlockSpec((128, N), lambda c: (c, 0))
    full = lambda shp: pl.BlockSpec(shp, lambda c: (0,) * len(shp))
    out = pl.pallas_call(
        _kernel,
        grid=(4,),
        in_specs=[pl.BlockSpec((L, 128), lambda c: (0, c))] + [par] * 6 + [
            pl.BlockSpec((128, 1), lambda c: (c, 0)),
            pl.BlockSpec((1, 128), lambda c: (0, c)),
            pl.BlockSpec((L // 4, D), lambda c: (c, 0)),
            full((D, 3 * D)), full((D, D)), full(_FU.shape), full(_FK.shape), full(_G.shape)],
        out_specs=pl.BlockSpec(memory_space=pl.ANY),
        out_shape=jax.ShapeDtypeStruct((L, 2 * D), BF16),
        scratch_shapes=[pltpu.VMEM((8 * 128, N), F32)] * 4 + [
            pltpu.VMEM((6, 128, N), F32),
            pltpu.VMEM(((NC + 1) * 128, Q), F32),
            pltpu.VMEM((3, NC, Q, 128), F32),
            pltpu.VMEM((3, NC, Q, 128), F32),
            pltpu.VMEM((NC, 2 * Q, 128), BF16),
            pltpu.VMEM((L, 128), BF16),
            pltpu.VMEM((L, D), BF16),
            pltpu.VMEM((4, 128, 128), F32),
            pltpu.VMEM((8, D), F32),
            pltpu.VMEM((D, D), BF16),
            pltpu.VMEM((4, L // 4, D), BF16),
            pltpu.SemaphoreType.DMA(()),
            pltpu.SemaphoreType.DMA((4,)),
        ],
        compiler_params=pltpu.CompilerParams(
            dimension_semantics=("arbitrary",), vmem_limit_bytes=100 * 1024 * 1024),
    )(A_u.reshape(L, D), A_A_re, A_A_im, A_B_re, A_B_im, A_C_re, A_C_im,
      A_log_dt.reshape(D, 1), A_Dskip.reshape(1, D), B_x.reshape(L, D), B_wqkv, B_wo,
      _FU, _FK, _G)
    return out.reshape(1, L, 2 * D)
```

```python
import jax
import jax.numpy as jnp
import numpy as np
import ml_dtypes
from jax import lax
import jax.experimental.pallas as pl
import jax.experimental.pallas.tpu as pltpu

L = 2048
D = 512
N = 128
Q = 128
NC = L // Q
F32 = jnp.float32
BF16 = jnp.bfloat16


def _consts():
    w = np.pi * (2 * np.arange(Q) + 1) / (2 * Q)
    s = np.arange(Q)
    fu = np.concatenate([np.cos(np.outer(w, s)), -np.sin(np.outer(w, s))], 0)
    g = fu.T / Q
    lr = np.arange(L).astype(np.float32).astype(ml_dtypes.bfloat16).astype(np.int64)
    fk = np.zeros((NC, 2 * Q, 2 * Q))
    for m in range(NC):
        for tau in range(-Q + 1, Q):
            l = Q * m + tau
            if l < 0:
                continue
            col = lr[l] - Q * (m - 1)
            if col == 2 * Q:
                col = 2 * Q - 1
            fk[m, :Q, col] += np.cos(w * tau)
            fk[m, Q:, col] -= np.sin(w * tau)
    b = ml_dtypes.bfloat16
    return fu.astype(b), fk.astype(b), g.astype(b)


_FU, _FK, _G = _consts()


def _cmul(a, b):
    return a[0] * b[0] - a[1] * b[1], a[0] * b[1] + a[1] * b[0]


def _csq(a):
    t = a[0] * a[1]
    return a[0] * a[0] - a[1] * a[1], t + t


def _phi(t):
    return jnp.where(t > 0, t + 1.0, jnp.exp(t)) + 1e-6


def _nt(a, b):
    return lax.dot_general(a, b, (((1,), (1,)), ((), ())), preferred_element_type=F32)


def _kernel(u_ref, are_ref, aim_ref, bre_ref, bim_ref, cre_ref, cim_ref, ldt_ref, dsk_ref,
            x_ref, wqkv_ref, wo_ref, fu_ref, fk_ref, g_ref, out_ref,
            t1r, t1i, t2r, t2i, mul_ref, kbuf, kf, uf, ybuf, ystage, pq_ref, kv_ref, z_ref,
            wc_ref, ostage, sem_y, sem_o):
    c = pl.program_id(0)
    RB = L // 4

    @pl.when(c == 0)
    def _():
        kv_ref[...] = jnp.zeros_like(kv_ref)
        z_ref[...] = jnp.zeros_like(z_ref)

    def bq(r):
        x = x_ref[r * 128:(r + 1) * 128, :]
        q = jnp.dot(x, wqkv_ref[:, 0:D], preferred_element_type=F32)
        pq_ref[pl.ds(pl.multiple_of(c * RB + r * 128, 128), 128), :] = _phi(q).astype(BF16)

    zacc, kvacc = {}, {}

    def bkv_pieces():
        for r in range(4):
            for hh in range(1):
                x = x_ref[r * 128:(r + 1) * 128, :]
                cs = slice(512 * hh, 512 * (hh + 1))
                pk = _phi(jnp.dot(x, wqkv_ref[:, D + 512 * hh:D + 512 * (hh + 1)],
                                  preferred_element_type=F32))
                zacc[hh] = zacc.get(hh, 0.0) + jnp.sum(pk.reshape(16, 8, 512), axis=0)
                pk = pk.astype(BF16)
                yield
                v = jnp.dot(x, wqkv_ref[:, 2 * D + 512 * hh:2 * D + 512 * (hh + 1)],
                            preferred_element_type=F32).astype(BF16)
                yield
                for t in range(4):
                    sl = slice(128 * t, 128 * (t + 1))
                    kvacc[2 * hh + t] = kvacc.get(2 * hh + t, 0.0) + lax.dot_general(
                        pk[:, sl], v[:, sl], (((0,), (0,)), ((), ())), preferred_element_type=F32)
                    yield

    bgen = bkv_pieces()

    def ufwd(m):
        r = jnp.dot(fu_ref[...], u_ref[m * Q:(m + 1) * Q, :], preferred_element_type=F32)
        uf[0, m] = r[:Q] + r[Q:]
        uf[1, m] = r[:Q]
        uf[2, m] = r[Q:]

    dt = jnp.exp(ldt_ref[...].astype(F32)).astype(BF16).astype(F32)
    lr = dt * are_ref[...].astype(F32)
    li = dt * aim_ref[...].astype(F32)
    e = jnp.exp(lr)
    a = (e * jnp.cos(li), e * jnp.sin(li))
    wv = _cmul((cre_ref[...].astype(F32), cim_ref[...].astype(F32)),
               (dt * bre_ref[...].astype(F32), dt * bim_ref[...].astype(F32)))
    pw = {1: a}
    p = a
    for k in range(1, 12):
        p = _csq(p)
        pw[2 ** k] = p
    p = (jnp.ones_like(lr), jnp.zeros_like(lr))
    b = wv
    for qq in range(8):
        t2r[qq * 128:(qq + 1) * 128, :] = p[0]
        t2i[qq * 128:(qq + 1) * 128, :] = p[1]
        t1r[qq * 128:(qq + 1) * 128, :] = b[0]
        t1i[qq * 128:(qq + 1) * 128, :] = b[1]
        if qq < 7:
            p = _cmul(p, a)
            b = _cmul(b, pw[128])
    for k, key in enumerate((8, 64, 1024)):
        mul_ref[2 * k] = pw[key][0]
        mul_ref[2 * k + 1] = pw[key][1]
    kl = wv[0] * pw[2048][0] - wv[1] * pw[2048][1]
    klast = jnp.sum(kl, axis=1, keepdims=True)

    def kgen(gi, _):
        for dd in range(8):
            if dd % 4 == 0:
                next(bgen, None)
            d = gi * 8 + dd
            row = lambda k: jnp.broadcast_to(mul_ref[k, pl.ds(d, 1), :], (8, N))
            m8, m64, m1024 = (row(0), row(1)), (row(2), row(3)), (row(4), row(5))
            st = pl.ds(d, 8, stride=128)
            p = (t2r[st, :], t2i[st, :])
            rows = [p]
            for _i in range(7):
                p = _cmul(p, m8)
                rows.append(p)
            e2 = jnp.concatenate(
                [jnp.concatenate([r[0] for r in rows], 0), jnp.concatenate([r[1] for r in rows], 0)],
                1).astype(BF16)
            b0 = (t1r[st, :], t1i[st, :])
            b1 = _cmul(b0, m1024)
            b2 = _cmul(b0, m64)
            b3 = _cmul(b1, m64)
            e1 = jnp.concatenate(
                [jnp.concatenate([b0[0], b1[0], b2[0], b3[0]], 0),
                 jnp.concatenate([-b0[1], -b1[1], -b2[1], -b3[1]], 0)], 1).astype(BF16)
            res = _nt(e1, e2)
            kbuf[pl.ds(d, NC, stride=128), :] = jnp.concatenate([res[:16], res[16:]], 1)
        return 0

    for gi in range(16):
        if gi % 4 == 0:
            bq(gi // 4)
        if gi % 4 == 2:
            for m in range(gi - 2, gi + 2):
                ufwd(m)
        kgen(gi, 0)

    lane = lax.broadcasted_iota(jnp.int32, (Q, Q), 1)

    kbuf[NC * Q:(NC + 1) * Q, :] = jnp.broadcast_to(klast, (Q, Q))

    def kfwd(it, prev):
        for mm in range(4):
            m = it * 4 + mm
            kj = kbuf[pl.ds(m * Q, Q), :]
            nxt = pltpu.roll(kbuf[pl.ds((m + 1) * Q, Q), :], Q - 1, 1)
            cur = (jnp.where(lane == Q - 1, nxt, kj) if m >= 2 else kj).astype(BF16)
            r = (_nt(fk_ref[m], jnp.concatenate([prev, cur], 1)) if m
                 else _nt(fk_ref[0, :, Q:], cur))
            prev = cur
            kf[0, m] = r[:Q]
            kf[1, m] = r[Q:] - r[:Q]
            kf[2, m] = r[Q:] + r[:Q]
        return prev

    prev = None
    for it in range(NC // 4):
        prev = kfwd(it, prev)

    def mac(fi):
        IB = 4
        for i0 in range(0, NC, IB):
            res = []
            for h in range(2):
                fs = pl.ds(fi * 16 + h * 8, 8)
                acc = {}
                kk = {}
                for j in range(i0 + IB - 1, -1, -1):
                    uu = [uf[t, j, fs, :] for t in range(3)]
                    for i in range(i0, i0 + IB):
                        if j <= i:
                            m = i - j
                            if m not in kk:
                                kk[m] = [kf[t, m, fs, :] for t in range(3)]
                            pr = [kk[m][t] * uu[t] for t in range(3)]
                            acc[i] = pr if i not in acc else [x_ + y_ for x_, y_ in zip(acc[i], pr)]
                res.append({i: (a_[0] - a_[2], a_[0] + a_[1]) for i, a_ in acc.items()})
            for i in range(i0, i0 + IB):
                for k in range(2):
                    ybuf[i, pl.ds(k * Q + fi * 16, 16), :] = jnp.concatenate(
                        [res[0][i][k], res[1][i][k]], 0).astype(BF16)

    for fi in range(8):
        mac(fi)
    for hh in range(1):
        z_ref[:, 512 * hh:512 * (hh + 1)] += zacc[hh]
    for t in range(4):
        kv_ref[t] += kvacc[t]

    def ycopy(cc):
        return pltpu.make_async_copy(
            ystage, out_ref.at[:, pl.ds(pl.multiple_of(cc * 128, 128), 128)], sem_y)

    @pl.when(c > 0)
    def _():
        ycopy(c - 1).wait()

    dsk = dsk_ref[...].astype(F32)
    for i in range(NC):
        y = jnp.dot(g_ref[...], ybuf[i], preferred_element_type=F32)
        ystage[i * Q:(i + 1) * Q, :] = (y + u_ref[i * Q:(i + 1) * Q, :].astype(F32) * dsk).astype(BF16)
    ycopy(c).start()

    @pl.when(c == 3)
    def _():
        r_i = lax.broadcasted_iota(jnp.int32, (128, 128), 0) // 16
        c_i = lax.broadcasted_iota(jnp.int32, (128, 128), 1) // 16
        msk = r_i == c_i
        z = jnp.sum(z_ref[...], axis=0, keepdims=True)
        zm, wc = [], []
        for t in range(4):
            sl = slice(128 * t, 128 * (t + 1))
            zt = jnp.broadcast_to(z[:, sl], (128, 128))
            zm.append(jnp.where(msk, zt, 0.0).astype(BF16))
            kvt = jnp.where(msk, kv_ref[t], 0.0).astype(BF16)
            wc.append(jnp.dot(kvt, wo_ref[sl, :], preferred_element_type=F32).astype(BF16))
        wcm = jnp.concatenate(wc, 0)
        wc_ref[...] = wcm
        for rb in range(4):
            for r in range(4):
                pq = pq_ref[rb * RB + r * 128:rb * RB + (r + 1) * 128, :]
                o = []
                for t in range(4):
                    pt = pq[:, 128 * t:128 * (t + 1)]
                    den = _nt(pt, zm[t]) + 1e-6
                    rc = pl.reciprocal(den, approx=True)
                    rc = rc * (2.0 - den * rc)
                    o.append((pt.astype(F32) * rc).astype(BF16))
                o = jnp.concatenate(o, 1)
                ostage[rb, r * 128:(r + 1) * 128, :] = jnp.dot(
                    o, wc_ref[...], preferred_element_type=F32).astype(BF16)
            pltpu.make_async_copy(ostage.at[rb], out_ref.at[rb * RB:(rb + 1) * RB, D:2 * D],
                                  sem_o.at[rb]).start()
        for rb in range(4):
            pltpu.make_async_copy(ostage.at[rb], out_ref.at[rb * RB:(rb + 1) * RB, D:2 * D],
                                  sem_o.at[rb]).wait()
        ycopy(c).wait()


@jax.jit
def pallas_concat_heads__ssm_conv_s4__linear_attn_block__prompt_kernel(
    A_u, A_A_re, A_A_im, A_B_re, A_B_im, A_C_re, A_C_im, A_log_dt, A_Dskip, B_x, B_wqkv, B_wo,
):
    par = pl.BlockSpec((128, N), lambda c: (c, 0))
    full = lambda shp: pl.BlockSpec(shp, lambda c: (0,) * len(shp))
    out = pl.pallas_call(
        _kernel,
        grid=(4,),
        in_specs=[pl.BlockSpec((L, 128), lambda c: (0, c))] + [par] * 6 + [
            pl.BlockSpec((128, 1), lambda c: (c, 0)),
            pl.BlockSpec((1, 128), lambda c: (0, c)),
            pl.BlockSpec((L // 4, D), lambda c: (c, 0)),
            full((D, 3 * D)), full((D, D)), full(_FU.shape), full(_FK.shape), full(_G.shape)],
        out_specs=pl.BlockSpec(memory_space=pl.ANY),
        out_shape=jax.ShapeDtypeStruct((L, 2 * D), BF16),
        scratch_shapes=[pltpu.VMEM((8 * 128, N), F32)] * 4 + [
            pltpu.VMEM((6, 128, N), F32),
            pltpu.VMEM(((NC + 1) * 128, Q), F32),
            pltpu.VMEM((3, NC, Q, 128), F32),
            pltpu.VMEM((3, NC, Q, 128), F32),
            pltpu.VMEM((NC, 2 * Q, 128), BF16),
            pltpu.VMEM((L, 128), BF16),
            pltpu.VMEM((L, D), BF16),
            pltpu.VMEM((4, 128, 128), F32),
            pltpu.VMEM((8, D), F32),
            pltpu.VMEM((D, D), BF16),
            pltpu.VMEM((4, L // 4, D), BF16),
            pltpu.SemaphoreType.DMA(()),
            pltpu.SemaphoreType.DMA((4,)),
        ],
        compiler_params=pltpu.CompilerParams(
            dimension_semantics=("arbitrary",), vmem_limit_bytes=100 * 1024 * 1024),
    )(A_u.reshape(L, D), A_A_re, A_A_im, A_B_re, A_B_im, A_C_re, A_C_im,
      A_log_dt.reshape(D, 1), A_Dskip.reshape(1, D), B_x.reshape(L, D), B_wqkv, B_wo,
      _FU, _FK, _G)
    return out.reshape(1, L, 2 * D)
```
